```python
import os as _os
_os.environ.setdefault("JAX_PLATFORMS", "cpu")
import jax
import jax.numpy as jnp

def _softmax(x, axis=-1):
    return jax.nn.softmax(x, axis=axis)
def _gelu(x):
    return jax.nn.gelu(x, approximate=True)
def _silu(x):
    return jax.nn.silu(x)
def _sigmoid(x):
    return jax.nn.sigmoid(x)
def _layernorm(x, axis=-1, eps=1e-5):
    m = jnp.mean(x, axis=axis, keepdims=True)
    v = jnp.var(x, axis=axis, keepdims=True)
    return (x - m) / jnp.sqrt(v + eps)
def _scatter_add(tgt, idx, src, axis=0):
    return tgt.at[idx].add(src)
def _segment_sum(src, seg, n):
    return jax.ops.segment_sum(src, seg, n)
class _Rng:
    def __init__(self, key):
        self._k = key
    def _next(self):
        self._k, sub = jax.random.split(self._k)
        return sub
    def normal(self, shape):
        return jax.random.normal(self._next(), shape, dtype=jnp.bfloat16)
    def randint(self, lo, hi, shape):
        return jax.random.randint(self._next(), shape, lo, hi, dtype=jnp.int32)
    def uniform(self, shape, lo=0.0, hi=1.0):
        return jax.random.uniform(self._next(), shape, jnp.bfloat16, lo, hi)
    def permutation(self, n):
        return jax.random.permutation(self._next(), n)


kernel_name = 'sequential_preLN__softmax_full_mha__dense_activation_squared_relu__prompt'

def setup_inputs():
    _rng = _Rng(jax.random.key(int.from_bytes(__import__("os").urandom(4), "little")))
    _w = (lambda a: (lambda t: t.astype(jnp.bfloat16) if jnp.issubdtype(t.dtype, jnp.floating) else t)(jnp.asarray(a)))
    def _A_setup():
        B, S, D = 1, 2048, 640
        return {
            "x": _w((lambda *s: _rng.normal(s) * 0.05)(B, S, D)),
            "wqkv": _w((lambda *s: _rng.normal(s) * 0.05)(D, 3 * D)),
            "wo": _w((lambda *s: _rng.normal(s) * 0.05)(D, D)),
        }
    _A_in = _A_setup()

    def _B_setup():
        B, S, D, F = 1, 2048, 640, 1536
        return {
            "x": _w((lambda *s: _rng.normal(s) * 0.05)(B, S, D)),
            "w1": _w((lambda *s: _rng.normal(s) * 0.05)(D, F)),
            "b1": _w((lambda *s: _rng.normal(s) * 0.05)(F)),
            "w2": _w((lambda *s: _rng.normal(s) * 0.05)(F, D)),
            "b2": _w((lambda *s: _rng.normal(s) * 0.05)(D)),
        }
    _B_in = _B_setup()

    return {
        "A_x": _A_in["x"],
        "A_wqkv": _A_in["wqkv"],
        "A_wo": _A_in["wo"],
        "B_x": _B_in["x"],
        "B_w1": _B_in["w1"],
        "B_b1": _B_in["b1"],
        "B_w2": _B_in["w2"],
        "B_b2": _B_in["b2"],
    }

def reference(A_x, A_wqkv, A_wo, B_x, B_w1, B_b1, B_w2, B_b2):
    def _A_ref(x, wqkv, wo):
        B, S, D = x.shape
        H = 32; Dh = D // H
        qkv = (lambda x, *d: x.transpose(*d))((x @ wqkv).reshape(B, S, 3, H, Dh), 2, 0, 3, 1, 4)
        q, k, v = qkv[0], qkv[1], qkv[2]
        scale = Dh ** -0.5
        scores = jnp.einsum("bhqd,bhkd->bhqk", q, k) * scale
        p = _softmax(scores, axis=-1)
        o = jnp.einsum("bhqk,bhkd->bhqd", p, v)
        return (lambda x, *d: x.transpose(*d))(o, 0, 2, 1, 3).reshape(B, S, D) @ wo

    def _B_ref(x, w1, b1, w2, b2):
        h = jnp.einsum("bsd,df->bsf", x, w1) + b1
        zero = jnp.zeros_like(h)
        r = jnp.where(h > zero, h, zero)
        h = r * r
        out = jnp.einsum("bsf,fd->bsd", h, w2) + b2
        return out

    x = A_x
    h = x + _A_ref(_layernorm(x, axis=-1), A_wqkv, A_wo)
    h2 = h + _B_ref(_layernorm(h, axis=-1), B_w1, B_b1, B_w2, B_b2)
    return h2
```

```python
import functools

import jax
import jax.numpy as jnp
import numpy as np
from jax import lax
import jax.experimental.pallas as pl
import jax.experimental.pallas.tpu as pltpu

S, D, H, DH, F = 2048, 640, 32, 20, 1536
LANES = 128
NB = D // LANES
TM = 512
NQ = 512
KC = 128
HG = 4
VR = 24
EPS = 1e-5
QSCALE = float(DH ** -0.5 * np.log2(np.e))
STRADDLE = [h for h in range(H) if (DH * h) // LANES != (DH * h + DH - 1) // LANES]
F32, BF16 = jnp.float32, jnp.bfloat16
NT = (((1,), (1,)), ((), ()))


def _mm(a, b):
    return jnp.dot(a, b, preferred_element_type=F32)


def _layernorm(v):
    mean = jnp.sum(v, axis=-1, keepdims=True) * (1.0 / D)
    c = v - mean
    var = jnp.sum(c * c, axis=-1, keepdims=True) * (1.0 / D)
    return c * lax.rsqrt(var + EPS)


def _head_block(h):
    blk = (DH * h) // LANES
    for j, hs in enumerate(STRADDLE):
        blk = jnp.where(h == hs, NB + j, blk)
    return blk


def _kernel(x_hbm, wqkv_hbm, wo_hbm, w1_hbm, b1_hbm, w2_hbm, b2_hbm, out_hbm,
            x_buf, wqkv_buf, wo_buf, w1_buf, b1_buf, w2_buf, b2_buf,
            q_buf, k_buf, vt_buf, ot_buf, s_buf, h_buf, hn_buf, out_buf, sems):
    n_chunks = S // TM

    def x_copy(c):
        rows = pl.ds(c * TM, TM)
        return pltpu.make_async_copy(x_hbm.at[0, rows], x_buf.at[rows], sems.at[c])

    def out_copy(c):
        rows = pl.ds(c * TM, TM)
        return pltpu.make_async_copy(out_buf.at[rows], out_hbm.at[0, rows], sems.at[n_chunks + c])

    base = 2 * n_chunks
    wqkv_copy = pltpu.make_async_copy(wqkv_hbm, wqkv_buf, sems.at[base])
    tail_copies = [
        pltpu.make_async_copy(src, dst, sems.at[base + 1 + j])
        for j, (src, dst) in enumerate(
            [(wo_hbm, wo_buf), (w1_hbm, w1_buf), (b1_hbm, b1_buf), (w2_hbm, w2_buf), (b2_hbm, b2_buf)])
    ]

    x_copy(0).start()
    wqkv_copy.start()
    for c in range(1, n_chunks):
        x_copy(c).start()
    for cp in tail_copies:
        cp.start()

    x_copy(0).wait()
    wqkv_copy.wait()

    def qkv_chunk(c, carry):
        @pl.when(c > 0)
        def _():
            x_copy(c).wait()

        rows = pl.ds(pl.multiple_of(c * TM, TM), TM)
        xn = _layernorm(x_buf[rows, :].astype(F32)).astype(BF16)
        hi = lax.broadcasted_iota(jnp.int32, (TM, LANES), 1) >= LANES // 2

        def split(y, dst):
            blocks = [y[:, b * LANES:(b + 1) * LANES] for b in range(NB)]
            for b in range(NB):
                dst[b, rows, :] = blocks[b].astype(BF16)
            for j, hs in enumerate(STRADDLE):
                b = (DH * hs) // LANES
                dst[NB + j, rows, :] = jnp.where(hi, blocks[b], blocks[b + 1]).astype(BF16)

        v = _mm(xn, wqkv_buf[:, 2 * D:3 * D])
        vt_buf[:, rows] = v.astype(BF16).astype(F32).T
        split(_mm(xn, wqkv_buf[:, 0:D]) * QSCALE, q_buf)
        split(_mm(xn, wqkv_buf[:, D:2 * D]), k_buf)
        return carry

    lax.fori_loop(0, n_chunks, qkv_chunk, 0)

    n_groups = H // HG
    n_steps = n_groups * (S // NQ)

    def attn_step(i_scores, i_out, m_cur):
        m_next = []
        o_prev = None
        if i_out is not None:
            g_out, c_out = i_out % n_groups, i_out // n_groups
            cols_out = pl.ds(pl.multiple_of(c_out * NQ, NQ), NQ)
        if i_scores is not None:
            g_sc, c_sc = i_scores % n_groups, i_scores // n_groups
            rows_sc = pl.ds(pl.multiple_of(c_sc * NQ, NQ), NQ)
        sub = lax.broadcasted_iota(jnp.int32, (VR, KC), 0)
        lane = lax.broadcasted_iota(jnp.int32, (NQ, LANES), 1)
        for u in range(HG):
            odd = u % 2
            if i_scores is not None:
                h = g_sc * HG + u
                blk = _head_block(h)
                in_head = ((lane - (DH * h) % LANES) & (LANES - 1)) < DH
                q = jnp.where(in_head, q_buf[blk, rows_sc, :].astype(F32), 0.0).astype(BF16)
            if i_out is not None:
                r0 = pl.multiple_of(g_out * (HG * DH) + (u * DH // 8) * 8, 8)
                is_one = (sub < VR - DH) if odd else (sub >= DH)
            m8 = acc = None
            for c in range(0, S, KC):
                if i_out is not None:
                    p = jnp.exp2(s_buf[u, c:c + KC, :] - m_cur[u]).astype(BF16)
                    vt = jnp.where(is_one, 1.0, vt_buf[pl.ds(r0, VR), c:c + KC])
                    d = _mm(vt, p)
                    acc = d if acc is None else acc + d
                if i_scores is not None:
                    s = lax.dot_general(k_buf[blk, c:c + KC, :], q, NT, preferred_element_type=F32)
                    s_buf[u, c:c + KC, :] = s
                    cm = jnp.max(s.reshape(KC // 8, 8, NQ), axis=0)
                    m8 = cm if m8 is None else jnp.maximum(m8, cm)
            if i_scores is not None:
                m_next.append(jnp.max(m8, axis=0, keepdims=True))
            if i_out is not None:
                denom = acc[0:1] if odd else acc[VR - 1:VR]
                o = acc * (1.0 / denom)
                if odd:
                    first = lax.broadcasted_iota(jnp.int32, (8, NQ), 0) < VR - DH
                    ot_buf[pl.ds(r0, 8), cols_out] = jnp.where(first, o_prev, o[0:8])
                    ot_buf[pl.ds(r0 + 8, VR - 8), cols_out] = o[8:]
                else:
                    ot_buf[pl.ds(r0, VR - 8), cols_out] = o[:VR - 8]
                    o_prev = o[VR - 8:]
        return tuple(m_next)

    m = attn_step(0, None, None)
    m = lax.fori_loop(0, n_steps - 1, lambda i, m: attn_step(i + 1, i, m), m)
    attn_step(None, n_steps - 1, m)

    for cp in tail_copies:
        cp.wait()

    def proj(c):
        rows = pl.ds(pl.multiple_of(c * TM, TM), TM)
        o = ot_buf[:, rows].T.astype(BF16)
        h = x_buf[rows, :].astype(F32) + _mm(o, wo_buf[...])
        return h, _layernorm(h).astype(BF16)

    def ffn(c, h, hn):
        rows = pl.ds(pl.multiple_of(c * TM, TM), TM)
        f = _mm(hn, w1_buf[...]) + b1_buf[...].astype(F32)[None, :]
        r = jnp.where(f > 0.0, f, 0.0)
        y = _mm((r * r).astype(BF16), w2_buf[...]) + b2_buf[...].astype(F32)[None, :]
        out_buf[rows, :] = (h + y).astype(BF16)

    h0, hn0 = proj(0)
    h_buf[...] = h0
    hn_buf[...] = hn0

    def tail_chunk(c, carry):
        h, hn = h_buf[...], hn_buf[...]
        h1, hn1 = proj(c + 1)
        ffn(c, h, hn)
        h_buf[...] = h1
        hn_buf[...] = hn1
        out_copy(c).start()
        return carry

    lax.fori_loop(0, n_chunks - 1, tail_chunk, 0)
    ffn(n_chunks - 1, h_buf[...], hn_buf[...])
    out_copy(n_chunks - 1).start()
    for c in range(n_chunks):
        out_copy(c).wait()


@jax.jit
def pallas_sequential_preLN__softmax_full_mha__dense_activation_squared_relu__prompt_kernel(
    A_x: jax.Array,
    A_wqkv: jax.Array,
    A_wo: jax.Array,
    B_x: jax.Array,
    B_w1: jax.Array,
    B_b1: jax.Array,
    B_w2: jax.Array,
    B_b2: jax.Array,
):
    del B_x
    n_blocks = NB + len(STRADDLE)
    scratch = [
        pltpu.VMEM((S, D), BF16), pltpu.VMEM((D, 3 * D), BF16), pltpu.VMEM((D, D), BF16),
        pltpu.VMEM((D, F), BF16), pltpu.VMEM((F,), BF16), pltpu.VMEM((F, D), BF16), pltpu.VMEM((D,), BF16),
        pltpu.VMEM((n_blocks, S, LANES), BF16), pltpu.VMEM((n_blocks, S, LANES), BF16),
        pltpu.VMEM((D, S), F32), pltpu.VMEM((D, S), F32), pltpu.VMEM((HG, S, NQ), F32),
        pltpu.VMEM((TM, D), F32), pltpu.VMEM((TM, D), BF16), pltpu.VMEM((S, D), BF16),
        pltpu.SemaphoreType.DMA((2 * (S // TM) + 6,)),
    ]
    any_spec = pl.BlockSpec(memory_space=pl.ANY)
    return pl.pallas_call(
        _kernel,
        out_shape=jax.ShapeDtypeStruct(A_x.shape, A_x.dtype),
        in_specs=[any_spec] * 7,
        out_specs=any_spec,
        scratch_shapes=scratch,
        compiler_params=pltpu.CompilerParams(vmem_limit_bytes=100 * 2**20),
    )(A_x, A_wqkv, A_wo, B_w1, B_b1, B_w2, B_b2)
```

```python
import jax
import jax.numpy as jnp
import numpy as np
from jax import lax
import jax.experimental.pallas as pl
import jax.experimental.pallas.tpu as pltpu


F32, BF16, I32 = jnp.float32, jnp.bfloat16, jnp.int32
S, D, H, DH, F = 2048, 640, 32, 20, 1536
EPS = 1e-5
QSCALE = float(DH ** -0.5 * np.log2(np.e))
SUM_MIN = 2.0 ** -60
ACC_MAX = 2.0 ** 100

LANES = 128
NB = D // LANES
TM = 512
N_CHUNKS = S // TM
HM = TM // 2
HD = 2 * LANES
HF = F // 2
LN_ROWS = 16
NQ = 512
NU = S // NQ
KC = 128
NP = S // KC
VR = 24
STRADDLE = [p for p in range(H // 2) if 2 * DH * p % LANES + 2 * DH > LANES]

VPU_KEYS = [[16 * int(x[j % len(x)]) for j in range(NP)]
            for x in "0011111211111112/11111112/11111112/11111112".split("/")]
VPU_ANY = [max(n[j] for n in VPU_KEYS) for j in range(NP)]
VPU_MAX = max(VPU_ANY)
PASSES = [(u, j) for u in range(NU) for j in range(NP)]

VPU_FIRST, VPU_LAST = 1.0, 0.0
VPU_LEAD, VPU_SPAN = 0.77, 0.9
VPU_PACED = range(1, DH, 6)
VPU_LANE = 256
KEY_TURN, VALUE_TURN, QUERY_PASS = 3, 1, 9
SPREAD_TURN, SPREAD_AHEAD = 3, 5
LN_PLAN = [int(n) for n in "0010101021212122"]
LN_ROW, LN_ROW_STEP, LN_LANE_STEP = 32, 64, 3
SUM_ROW_STEP = 56

A_SUMS = (1, 2, 5, 6, 7)
B_SUMS = (1, 3, 4, 6, 7)


def _mm(a, b):
    return jnp.dot(a, b, preferred_element_type=F32)


def _after(never, earlier, value):
    return jnp.where(never, earlier, value)


def _layernorm(v):
    mean = jnp.sum(v, axis=-1, keepdims=True) * (1.0 / D)
    c = v - mean
    var = jnp.sum(c * c, axis=-1, keepdims=True) * (1.0 / D)
    return c * lax.rsqrt(var + EPS)


def _rows(i, n):
    return pl.ds(i * n, n) if isinstance(i, int) else pl.ds(pl.multiple_of(i * n, n), n)


def _to_words(v):
    return pltpu.bitcast(v.astype(BF16), I32)


def _from_words(w):
    return pltpu.bitcast(w, BF16)


def _left(i, a):
    return {1: lambda: a(0, 0) + a(1, 1), 2: lambda: a(1, 0) + a(1, 1), 3: lambda: a(0, 0), 4: lambda: a(1, 1),
            5: lambda: a(0, 0) + a(0, 1), 6: lambda: a(1, 0) - a(0, 0), 7: lambda: a(0, 1) - a(1, 1)}[i]()


def _right(i, b):
    return {1: lambda: b(0, 0) + b(1, 1), 2: lambda: b(0, 0), 3: lambda: b(0, 1) - b(1, 1),
            4: lambda: b(1, 0) - b(0, 0), 5: lambda: b(1, 1), 6: lambda: b(0, 0) + b(0, 1),
            7: lambda: b(1, 0) + b(1, 1)}[i]()


def _strassen(product, base, emit):
    m5 = product(5)
    m3 = product(3)
    emit(0, 1, base(0, 1) + m5 + m3)
    m4 = product(4)
    c11 = base(0, 0) + m4 - m5
    m2 = product(2)
    emit(1, 0, base(1, 0) + m2 + m4)
    c22 = base(1, 1) + m3 - m2
    m1 = product(1)
    c11, c22 = c11 + m1, c22 + m1
    emit(0, 0, c11 + product(7))
    emit(1, 1, c22 + product(6))


def _vpu_jobs():
    blocks = [(u, j, r) for u, j in PASSES for r in range(KC - VPU_KEYS[u][j], KC, 16)]
    jobs = {}
    for n, block in enumerate(blocks):
        at = VPU_FIRST + (len(PASSES) - 1 + VPU_LAST - VPU_FIRST) * n / (len(blocks) - 1) + 1e-6
        jobs.setdefault(min(int(at), len(PASSES) - 1), []).append((*block, at - VPU_LEAD))
    return jobs


def _scratch_shapes():
    shapes = dict(
        x_buf=pltpu.VMEM((S, D), BF16), wqkv_buf=pltpu.VMEM((3, D, D), BF16), wo_buf=pltpu.VMEM((D, D), BF16),
        w1_buf=pltpu.VMEM((D, F), BF16), b1_buf=pltpu.VMEM((F,), BF16),
        w2_buf=pltpu.VMEM((F, D), BF16), b2_buf=pltpu.VMEM((D,), BF16),
        k_raw=pltpu.VMEM((TM // 2, D), I32),
        xn_buf=pltpu.VMEM((TM, D), BF16), xs_buf=pltpu.VMEM((5, HM, HD), BF16),
        sqk_buf=pltpu.VMEM((5, HD, D), BF16), sv_buf=pltpu.VMEM((5, HD, HD), BF16),
        so_buf=pltpu.VMEM((5, HD, HD), BF16), s1_buf=pltpu.VMEM((5, HD, HF), BF16),
        s2_buf=pltpu.VMEM((5, HF, HD), BF16),
        qt_buf=pltpu.VMEM((H, VR, S), F32), k_buf=pltpu.VMEM((NB + len(STRADDLE), S // 2, LANES), I32),
        vt_buf=pltpu.VMEM((H, VR, S), F32), ot_buf=pltpu.VMEM((H, VR, S), F32),
        h_buf=pltpu.VMEM((TM, D), F32), out_buf=pltpu.VMEM((S, D), BF16),
        kx_buf=pltpu.VMEM((H // 2, NP * VPU_MAX, LANES), F32), s_buf=pltpu.VMEM((S, NQ), F32),
        sems=pltpu.SemaphoreType.DMA((2 * N_CHUNKS + 11,)))
    for side in "01":
        shapes.update({"q_cur" + side: pltpu.VMEM((VR, S), F32), "k_cur" + side: pltpu.VMEM((S // 2, LANES), I32),
                       "v_cur" + side: pltpu.VMEM((VR, S), F32),
                       "kb_buf" + side: pltpu.VMEM((DH, sum(VPU_ANY), LANES), F32)})
    shapes.update(p_buf=pltpu.VMEM((NU, S, NQ), F32), range_buf=pltpu.VMEM((2, 8, NQ), F32))
    return list(shapes.values())


def _kernel(x_hbm, wqkv_hbm, wo_hbm, w1_hbm, b1_hbm, w2_hbm, b2_hbm, out_hbm,
            x_buf, wqkv_buf, wo_buf, w1_buf, b1_buf, w2_buf, b2_buf, k_raw, xn_buf, xs_buf,
            sqk_buf, sv_buf, so_buf, s1_buf, s2_buf, qt_buf, k_buf, vt_buf, ot_buf, h_buf, out_buf,
            kx_buf, s_buf, sems, q_cur0, k_cur0, v_cur0, kb_buf0, q_cur1, k_cur1, v_cur1, kb_buf1,
            p_buf, range_buf):
    q_cur, k_cur, v_cur, kb_buf = (q_cur0, q_cur1), (k_cur0, k_cur1), (v_cur0, v_cur1), (kb_buf0, kb_buf1)

    def x_copy(c):
        return pltpu.make_async_copy(x_hbm.at[0, _rows(c, TM)], x_buf.at[_rows(c, TM)], sems.at[c])

    def out_copy(c):
        return pltpu.make_async_copy(out_buf.at[_rows(c, TM)], out_hbm.at[0, _rows(c, TM)], sems.at[N_CHUNKS + c])

    copies = [(wqkv_hbm.at[:, pl.ds(j * D, D)], wqkv_buf.at[j]) for j in range(3)]
    copies += [(wo_hbm, wo_buf), (w1_hbm, w1_buf), (b1_hbm, b1_buf), (w2_hbm, w2_buf), (b2_hbm, b2_buf)]
    copies += [(out_buf.at[rows, cols], out_hbm.at[0, rows, cols]) for rows, cols in [
        (pl.ds(S - TM, HM), pl.ds(HD, D - HD)), (pl.ds(S - HM, HM), pl.ds(0, HD)),
        (pl.ds(S - TM, HM), pl.ds(0, HD)), (pl.ds(S - HM, HM), pl.ds(HD, D - HD))]]
    copies = [pltpu.make_async_copy(src, dst, sems.at[2 * N_CHUNKS - 1 + n]) for n, (src, dst) in enumerate(copies)]
    (wq_copy, wk_copy, wv_copy), tail_copies, last_copies = copies[:3], copies[3:8], copies[8:]

    def qk_block(r, c):
        return wqkv_buf.at[c, r * HD:(r + 1) * HD, :]

    def v_block(r, c):
        return wqkv_buf.at[2, r * HD:(r + 1) * HD, c * HD:(c + 1) * HD]

    def wo_block(r, c):
        return wo_buf.at[r * HD:(r + 1) * HD, c * HD:(c + 1) * HD]

    def w1_block(r, c):
        return w1_buf.at[r * HD:(r + 1) * HD, c * HF:(c + 1) * HF]

    def w2_block(r, c):
        return w2_buf.at[r * HF:(r + 1) * HF, c * HD:(c + 1) * HD]

    def weight_sums(dst, block):
        _, n_rows, n_cols = dst.shape

        def job(r, t):
            rows, cols = slice(r, r + 16), slice(t, min(t + HD, n_cols))

            def run(never, earlier):
                b = {(i, j): block(i, j).at[rows, cols][...].astype(F32) for i in range(2) for j in range(2)}
                for i in range(2):
                    reps = b[i, i].shape[1] // LANES
                    b[i, i] = _after(never, jnp.concatenate([earlier[0:16, 0:LANES]] * reps, axis=1), b[i, i])
                for i in B_SUMS:
                    dst[B_SUMS.index(i), rows, cols] = _right(i, lambda y, z: b[y, z]).astype(BF16)
            return run

        return [job(r, t) for r in range(0, n_rows, 16) for t in range(0, n_cols, HD)]

    def weights(i, sums, block):
        return sums[B_SUMS.index(i)] if i in B_SUMS else _right(i, block)[...]

    def normed(i):
        if i in A_SUMS:
            return xs_buf[A_SUMS.index(i)]
        return _left(i, lambda r, c: xn_buf[r * HM:(r + 1) * HM, c * HD:(c + 1) * HD])

    def norm_rows(load, r, sums=A_SUMS):
        halves = [_layernorm(load(half * HM + r)) for half in range(2)]
        out = [(xn_buf.at[pl.ds(half * HM + r, LN_ROWS)], halves[half].astype(BF16)) for half in range(2)]
        for i in sums:
            out.append((xs_buf.at[A_SUMS.index(i), pl.ds(r, LN_ROWS)],
                        _left(i, lambda a, b: halves[a][:, b * HD:(b + 1) * HD]).astype(BF16)))
        return out

    def flush(writes):
        for ref, val in writes:
            ref[...] = val

    def x_rows(c, never=None, earlier=None):
        def load(r):
            v = x_buf[pl.ds(pl.multiple_of(c * TM + r, LN_ROWS), LN_ROWS), :].astype(F32)
            if earlier is not None:
                v = jnp.concatenate([_after(never, earlier, v[:, :LANES]), v[:, LANES:]], axis=1)
            return v
        return load

    def key_block(p):
        b = 2 * DH * p // LANES
        for n, straddling in enumerate(STRADDLE):
            if isinstance(p, int):
                b = NB + n if p == straddling else b
            else:
                b = jnp.where(p == straddling, NB + n, b)
        return b

    def rotate_pair(keys, p):
        shift = (LANES - 2 * DH * p % LANES) % LANES
        return keys if isinstance(shift, int) and shift == 0 else pltpu.roll(keys, shift, 1)

    def put_keys(c, half, k_words):
        upper = lax.broadcasted_iota(I32, (HM // 2, LANES), 1) >= LANES // 2
        blocks = [k_words[:, b * LANES:(b + 1) * LANES] for b in range(NB)]
        blocks += [jnp.where(upper, blocks[2 * DH * p // LANES], blocks[2 * DH * p // LANES + 1]) for p in STRADDLE]
        for b, block in enumerate(blocks):
            k_buf[b, _rows(2 * c + half, HM // 2), :] = block
            ends = jnp.concatenate(
                [block[((j + 1) * KC - VPU_MAX) // 2:(j + 1) * KC // 2] for j in range(HM // KC)], axis=0)
            for p in range(H // 2):
                if key_block(p) == b:
                    kx_buf[p, _rows(2 * c + half, VPU_MAX * HM // KC), :] = _from_words(rotate_pair(ends, p)).astype(F32)

    def put_values(c, half, *v):
        rows = _rows(2 * c + half, HM)
        sub = lax.broadcasted_iota(I32, (8, HM), 0)
        vt = jnp.concatenate([part.astype(BF16).astype(F32).T for part in v], axis=0)
        for h in range(H):
            r0 = h * DH // 8 * 8
            if h % 2 == 0:
                vt_buf[h, 0:16, rows] = vt[r0:r0 + 16]
                vt_buf[h, 16:24, rows] = jnp.where(sub < 4, vt[r0 + 16:r0 + 24], 1.0)
            else:
                vt_buf[h, 0:8, rows] = jnp.where(sub < 4, 1.0, vt[r0:r0 + 8])
                vt_buf[h, 8:24, rows] = vt[r0 + 8:r0 + 24]

    def put_queries(c, half, q):
        qt = (q * QSCALE).T
        for h in range(H):
            qt_buf[h, :, _rows(2 * c + half, HM)] = jnp.concatenate(
                [qt[h * DH:(h + 1) * DH], jnp.zeros((VR - DH, HM), F32)], axis=0)

    x_copy(0).start()
    wk_copy.start()
    x_copy(0).wait()
    for r in range(0, HM, LN_ROWS):
        flush(norm_rows(x_rows(0), r, sums=()))
    wk_copy.wait()
    for cp in (wq_copy, wv_copy, x_copy(1)):
        cp.start()

    off = jnp.max(jnp.square(xn_buf[0:16, 0:LANES].astype(F32))) < 0.0
    k_raw[...] = _to_words(_mm(xn_buf[...], wqkv_buf[1]))
    wq_copy.wait()
    for c in range(2, N_CHUNKS):
        x_copy(c).start()
    q = _mm(xn_buf[...], wqkv_buf[0])
    h_buf[...] = q
    for half in range(2):
        put_keys(0, half, k_raw[half * HM // 2:(half + 1) * HM // 2, :])
    for n, job in enumerate(weight_sums(sqk_buf, qk_block)):
        job(off, q[n * SUM_ROW_STEP % (TM - 16) // 8 * 8:, n * NB // 48 * LANES:])
    wv_copy.wait()
    x_copy(1).wait()
    v = _mm(xn_buf[...], wqkv_buf[2])
    for half in range(2):
        put_queries(0, half, h_buf[half * HM:(half + 1) * HM, :])
    for n, job in enumerate(weight_sums(sv_buf, v_block)):
        job(off, v[n * SUM_ROW_STEP % (TM - 16) // 8 * 8:, n * NB // 16 * LANES:])
    writes = []
    for r in range(0, HM, LN_ROWS):
        writes += norm_rows(x_rows(1), r)
    for half in range(2):
        put_values(0, half, v[half * HM:(half + 1) * HM])
    flush(writes)
    for c in range(2, N_CHUNKS):
        x_copy(c).wait()
    for cp in tail_copies:
        cp.start()

    def qkv_chunk(c, carry):
        never = c < 0
        c_next = jnp.minimum(c + 1, N_CHUNKS - 1)
        todo, counts, writes = list(range(0, HM, LN_ROWS)), list(LN_PLAN), []

        def normalize_after(m):
            for k in range(counts.pop(0)):
                r, t = LN_ROW + k * LN_ROW_STEP, k * LN_LANE_STEP * LANES % m.shape[1]
                writes.extend(norm_rows(x_rows(c_next, never, m[r:r + LN_ROWS, t:t + LANES]), todo.pop(0)))
            return m

        v = {}
        rest = normalize_after(_mm(xn_buf[:, 2 * HD:], wqkv_buf[2, 2 * HD:, :2 * HD]))
        _strassen(lambda i: normalize_after(_mm(normed(i), weights(i, sv_buf, v_block))),
                  lambda r, col: rest[r * HM:(r + 1) * HM, col * HD:(col + 1) * HD],
                  lambda r, col, val: v.update({(r, col): val}))
        rest = normalize_after(_mm(
            xn_buf[:, 2 * HD:], jnp.concatenate([wqkv_buf[0, 2 * HD:, :], wqkv_buf[1, 2 * HD:, :]], axis=1)))
        _strassen(lambda i: normalize_after(_mm(normed(i), weights(i, sqk_buf, qk_block))),
                  lambda r, col: rest[r * HM:(r + 1) * HM, col * D:(col + 1) * D],
                  lambda r, col, val: put_keys(c, r, _to_words(val)) if col else put_queries(c, r, val))
        last = _mm(xn_buf[...], wqkv_buf[2, :, 2 * HD:])
        for r in range(2):
            put_values(c, r, v[r, 0], v[r, 1], last[r * HM:(r + 1) * HM])
        assert not todo
        flush(writes)
        return carry

    lax.fori_loop(1, N_CHUNKS, qkv_chunk, 0)

    vpu_jobs = _vpu_jobs()

    def spread_keys(side, pair, j):
        n = sum(VPU_ANY[:j])
        keys = kx_buf[pair, (j + 1) * VPU_MAX - VPU_ANY[j]:(j + 1) * VPU_MAX, :]
        for d in range(DH):
            kb_buf[side][d, n:n + VPU_ANY[j], :] = jnp.broadcast_to(
                keys[:, side * DH + d:side * DH + d + 1], (VPU_ANY[j], LANES))

    def attend(h, side, score=True, after_first_unit=None):
        scores, waiting = [], {}
        lo = hi = None
        if score:
            h_next = jnp.minimum(h + 1, H - 1)
            never = h < 0
        for g, (u, j) in enumerate(PASSES):
            cols, keys = slice(u * NQ, (u + 1) * NQ), slice(j * KC, (j + 1) * KC)
            n = KC - VPU_KEYS[u][j]
            if score:
                if j == 0:
                    qt = q_cur[side][:, cols].astype(BF16)
                s = _mm(_from_words(k_cur[side][j * KC // 2:(j * KC + n) // 2, :])[:, :VR], qt)
                scores.append(s)
                if u == (j + KEY_TURN) % NU:
                    used = slice(j * KC // 2, ((j + 1) * KC - min(n_vpu[j] for n_vpu in VPU_KEYS)) // 2)
                    if side:
                        k_cur[0][used, :] = rotate_pair(k_buf[key_block(h_next // 2), used, :], h_next // 2)
                    else:
                        k_cur[1][used, :] = pltpu.roll(k_cur[0][used, :], LANES - DH, 1)
                if j == QUERY_PASS:
                    q_cur[1 - side][:, cols] = qt_buf[h_next, :, cols]
            pv = _mm(v_cur[side][:, keys], p_buf[u, keys, :])
            acc = pv if j == 0 else acc + pv
            if score and u == (j + VALUE_TURN) % NU:
                v_cur[1 - side][:, keys] = vt_buf[h, :, keys]
            flush(waiting.pop(g, []))
            if j == NP - 1:
                ot_buf[h - 1, :, cols] = acc
                top = jnp.maximum(jnp.maximum(jnp.abs(acc[0:8]), jnp.abs(acc[8:16])), jnp.abs(acc[16:24]))
                sub = lax.broadcasted_iota(I32, (8, NQ), 0)
                total = jnp.where(sub >= 4, acc[16:24], ACC_MAX) if side else jnp.where(sub < 4, acc[0:8], ACC_MAX)
                lo = total if lo is None else jnp.minimum(lo, total)
                hi = top if hi is None else jnp.maximum(hi, top)
            if g == NP and after_first_unit:
                after_first_unit()
            if not score:
                continue
            for uu, jj, r, time in vpu_jobs.get(g, []):
                first = sum(VPU_ANY[:jj]) + r - (KC - VPU_ANY[jj])
                val = None
                for d in range(DH):
                    kb = kb_buf[side][d, first:first + 16, :]
                    when = time + (d - VPU_PACED[0]) / DH * VPU_SPAN
                    if d in VPU_PACED and when >= 0:
                        earlier = scores[min(int(when), g)]
                        row = int(when % 1 * (earlier.shape[0] - 8)) // 8 * 8
                        kb = _after(never, earlier[row:row + 16, VPU_LANE:VPU_LANE + LANES], kb)
                    term = jnp.concatenate(
                        [kb * q_cur[side][d:d + 1, t:t + LANES] for t in range(uu * NQ, (uu + 1) * NQ, LANES)], axis=1)
                    val = term if val is None else val + term
                write = (p_buf.at[uu, jj * KC + r:jj * KC + r + 16, :], jnp.exp2(val))
                if PASSES.index((uu, jj)) <= g:
                    flush([write])
                else:
                    waiting.setdefault(PASSES.index((uu, jj)), []).append(write)
            p_buf[u, j * KC:j * KC + n, :] = jnp.exp2(s)
            ahead = (j + SPREAD_AHEAD) % NP
            if (ahead + SPREAD_TURN) % NU == u:
                spread_keys(1 - side, h_next // 2, ahead)
        assert not waiting
        range_buf[0] = jnp.minimum(range_buf[0], lo)
        range_buf[1] = jnp.maximum(range_buf[1], hi)

    def attend_shifted(i, carry):
        h, cols = i // NU, _rows(i % NU, NQ)
        qt = qt_buf[h, :, cols].astype(BF16)

        def score(j, m):
            keys = pltpu.roll(k_buf[key_block(h // 2), _rows(j, KC // 2), :], (LANES - h * DH % LANES) % LANES, 1)
            s = _mm(_from_words(keys)[:, :VR], qt)
            s_buf[_rows(j, KC), :] = s
            return jnp.maximum(m, jnp.max(s.reshape(KC // 8, 8, NQ), axis=0))

        m = lax.fori_loop(0, NP, score, jnp.full((8, NQ), -jnp.inf, F32))
        m = jnp.max(m, axis=0, keepdims=True)

        def weigh(j, acc):
            return acc + _mm(vt_buf[h, :, _rows(j, KC)], jnp.exp2(s_buf[_rows(j, KC), :] - m))

        ot_buf[h, :, cols] = lax.fori_loop(0, NP, weigh, jnp.zeros((VR, NQ), F32))
        return carry

    for cp in tail_copies:
        cp.wait()
    off = jnp.max(jnp.square(qt_buf[0, 0:8, 0:LANES])) < 0.0
    jobs = weight_sums(so_buf, wo_block) + weight_sums(s1_buf, w1_block) + weight_sums(s2_buf, w2_block)
    n_jobs = len(jobs)
    for g, (u, j) in enumerate(PASSES):
        if j == 0:
            qt = qt_buf[0, :, u * NQ:(u + 1) * NQ].astype(BF16)
        s = _mm(_from_words(k_buf[0, j * KC // 2:(j + 1) * KC // 2, :])[:, :VR], qt)
        p_buf[u, j * KC:(j + 1) * KC, :] = jnp.exp2(s)
        while jobs and len(jobs) > n_jobs * (1 - (g + 3) / len(PASSES)):
            jobs.pop(0)(off, s[len(jobs) % 2 * SUM_ROW_STEP:])
    for j in range(NP):
        spread_keys(1, 0, j)
    k_cur[1][...] = pltpu.roll(k_buf[0], LANES - DH, 1)
    q_cur[1][...] = qt_buf[1]
    v_cur[1][...] = vt_buf[0]
    range_buf[0] = jnp.full((8, NQ), ACC_MAX, F32)
    range_buf[1] = jnp.zeros((8, NQ), F32)

    def head(h, carry):
        lax.cond(h % 2 == 1, lambda: attend(h, 1), lambda: attend(h, 0))
        return carry

    lax.fori_loop(1, H, head, None)

    def attention_out(c, n):
        rows = _rows(c, n)
        sub = lax.broadcasted_iota(I32, (8, n), 0)
        parts = []
        for h in range(0, H, 2):
            even, odd = ot_buf[h, :, rows], ot_buf[h + 1, :, rows]
            even = even * (1.0 / even[VR - 1:VR])
            odd = odd * (1.0 / odd[0:1])
            parts += [even[0:16], jnp.where(sub < 4, even[16:24], odd[0:8]), odd[8:24]]
        return jnp.concatenate(parts, axis=0).T

    def project(c):
        o = attention_out(c, TM)
        x = x_buf[_rows(c, TM), :].astype(F32)
        last = x[:, 2 * HD:] + _mm(o.astype(BF16), wo_buf[:, 2 * HD:])
        rest = x[:, :2 * HD] + _mm(o[:, 2 * HD:].astype(BF16), wo_buf[2 * HD:, :2 * HD])
        h = {}
        _strassen(lambda i: _mm(_left(i, lambda r, col: o[r * HM:(r + 1) * HM, col * HD:(col + 1) * HD]).astype(BF16),
                                weights(i, so_buf, wo_block)),
                  lambda r, col: rest[r * HM:(r + 1) * HM, col * HD:(col + 1) * HD],
                  lambda r, col, val: h.update({(r, col): val}))
        return jnp.concatenate(
            [jnp.concatenate([h[r, 0], h[r, 1], last[r * HM:(r + 1) * HM]], axis=1) for r in range(2)], axis=0)

    def ffn(c, is_last):
        act = {}

        def activate(r, col, f):
            f = jnp.where(f > 0.0, f, 0.0)
            act[r, col] = f * f

        rest = _mm(xn_buf[:, 2 * HD:], w1_buf[2 * HD:, :]) + b1_buf[...].astype(F32)[None, :]
        _strassen(lambda i: _mm(normed(i), weights(i, s1_buf, w1_block)),
                  lambda r, col: rest[r * HM:(r + 1) * HM, col * HF:(col + 1) * HF], activate)
        todo, writes = [], []
        if not is_last:
            h_next = project(c + 1)
            todo = list(range(0, HM, LN_ROWS))
        b2 = b2_buf[...].astype(F32)[None, :]
        for r in range(2):
            last = (_mm(act[r, 1 - r].astype(BF16), w2_buf[(1 - r) * HF:(2 - r) * HF, 2 * HD:])
                    + _mm(act[r, r].astype(BF16), w2_buf[r * HF:(r + 1) * HF, 2 * HD:]))
            out_buf[_rows(2 * c + r, HM), 2 * HD:] = (
                h_buf[r * HM:(r + 1) * HM, 2 * HD:] + b2[:, 2 * HD:] + last).astype(BF16)

        def product(i):
            m = _mm(_left(i, lambda r, col: act[r, col]).astype(BF16), weights(i, s2_buf, w2_block))

            def load(r):
                v = h_next[r:r + LN_ROWS]
                return jnp.concatenate([_after(c < 0, m[:LN_ROWS, :LANES], v[:, :LANES]), v[:, LANES:]], axis=1)

            for _ in range(3):
                if todo:
                    writes.extend(norm_rows(load, todo.pop(0)))
            return m

        def put_out(r, col, val):
            out_buf[_rows(2 * c + r, HM), col * HD:(col + 1) * HD] = val.astype(BF16)
            if is_last and (r, col) == (1, 0):
                for cp in last_copies[:2]:
                    cp.start()

        _strassen(product,
                  lambda r, col: h_buf[r * HM:(r + 1) * HM, col * HD:(col + 1) * HD] + b2[:, col * HD:(col + 1) * HD],
                  put_out)
        assert not todo
        if not is_last:
            h_buf[...] = h_next
            flush(writes)

    h_first = []
    attend(H, 0, score=False, after_first_unit=lambda: h_first.append(project(0)))
    h_buf[...] = h_first[0]
    writes = []
    for r in range(0, HM, LN_ROWS):
        writes += norm_rows(lambda r0: h_first[0][r0:r0 + LN_ROWS], r)
    flush(writes)
    safe = jnp.logical_and(range_buf[0] >= SUM_MIN, range_buf[1] <= ACC_MAX)

    @pl.when(jnp.max(jnp.where(safe, 0.0, 1.0)) > 0.0)
    def _():
        lax.fori_loop(0, H * NU, attend_shifted, 0)

        def project_again(i, carry):
            rows = _rows(i, LANES)
            h_buf[rows, :] = x_buf[rows, :].astype(F32) + _mm(attention_out(i, LANES).astype(BF16), wo_buf[...])
            return carry

        def normalize_again(i, carry):
            flush(norm_rows(lambda r: h_buf[pl.ds(r, LN_ROWS), :], pl.multiple_of(i * LN_ROWS, LN_ROWS)))
            return carry

        lax.fori_loop(0, TM // LANES, project_again, 0)
        lax.fori_loop(0, HM // LN_ROWS, normalize_again, 0)

    def ffn_chunk(c, carry):
        ffn(c, False)
        out_copy(c).start()
        return carry

    lax.fori_loop(0, N_CHUNKS - 1, ffn_chunk, 0)
    ffn(N_CHUNKS - 1, True)
    for cp in last_copies[2:]:
        cp.start()
    for cp in [out_copy(c) for c in range(N_CHUNKS - 1)] + last_copies:
        cp.wait()


@jax.jit
def pallas_sequential_preLN__softmax_full_mha__dense_activation_squared_relu__prompt_kernel(
    A_x: jax.Array,
    A_wqkv: jax.Array,
    A_wo: jax.Array,
    B_x: jax.Array,
    B_w1: jax.Array,
    B_b1: jax.Array,
    B_w2: jax.Array,
    B_b2: jax.Array,
):
    del B_x
    any_spec = pl.BlockSpec(memory_space=pl.ANY)
    return pl.pallas_call(
        _kernel,
        out_shape=jax.ShapeDtypeStruct(A_x.shape, A_x.dtype),
        in_specs=[any_spec] * 7,
        out_specs=any_spec,
        scratch_shapes=_scratch_shapes(),
        compiler_params=pltpu.CompilerParams(
            vmem_limit_bytes=110 * 2**20,
            flags={"XLA_TPU_EVENLY_DISTRIBUTE_CRITICAL_NODES": True}),
    )(A_x, A_wqkv, A_wo, B_w1, B_b1, B_w2, B_b2)
```

```python
import jax
import jax.numpy as jnp
import numpy as np
from jax import lax
import jax.experimental.pallas as pl
import jax.experimental.pallas.tpu as pltpu


F32, BF16, I32 = jnp.float32, jnp.bfloat16, jnp.int32
S, D, H, DH, F = 2048, 640, 32, 20, 1536
EPS = 1e-5
QSCALE = float(DH ** -0.5 * np.log2(np.e))
SUM_MIN = 2.0 ** -60
ACC_MAX = 2.0 ** 100

LANES = 128
NB = D // LANES
TM = 512
N_CHUNKS = S // TM
HM = TM // 2
HD = 2 * LANES
HF = F // 2
LN_ROWS = 16
NQ = 512
NU = S // NQ
KC = 128
NP = S // KC
VR = 24
STRADDLE = [p for p in range(H // 2) if 2 * DH * p % LANES + 2 * DH > LANES]

VPU_KEYS = [[16 * int(x[j % len(x)]) for j in range(NP)]
            for x in "0011111211111112/11111112/11111112/11111112".split("/")]
VPU_ANY = [max(n[j] for n in VPU_KEYS) for j in range(NP)]
VPU_MAX = max(VPU_ANY)
PASSES = [(u, j) for u in range(NU) for j in range(NP)]

VPU_FIRST, VPU_LAST = 1.0, 0.0
VPU_LEAD, VPU_SPAN = 0.77, 0.9
VPU_NUDGE = [(ord(ch) - ord("m")) / 20 for ch in
             "jmmjmmmmmmlmnkkmmmmommnmmmmmmnmmnlmmmmmklmommmmmmmmmmimmllmmjmqmnmmmom"]
VPU_PACED = range(1, DH, 6)
VPU_LANE = 256
KEY_TURN, VALUE_TURN, QUERY_PASS = 2, 1, 9
SPREAD_TURN, SPREAD_AHEAD = 2, 5
LN_PLAN = [int(n) for n in "0010101021212122"]
LN_ROW, LN_ROW_STEP, LN_LANE_STEP = 32, 64, 3
SUM_ROW_STEP = 56

A_SUMS = (1, 2, 5, 6, 7)
B_SUMS = (1, 3, 4, 6, 7)


def _mm(a, b):
    return jnp.dot(a, b, preferred_element_type=F32)


def _after(never, earlier, value):
    return jnp.where(never, earlier, value)


def _layernorm(v):
    mean = jnp.sum(v, axis=-1, keepdims=True) * (1.0 / D)
    c = v - mean
    var = jnp.sum(c * c, axis=-1, keepdims=True) * (1.0 / D)
    return c * lax.rsqrt(var + EPS)


def _rows(i, n):
    return pl.ds(i * n, n) if isinstance(i, int) else pl.ds(pl.multiple_of(i * n, n), n)


def _to_words(v):
    return pltpu.bitcast(v.astype(BF16), I32)


def _from_words(w):
    return pltpu.bitcast(w, BF16)


def _left(i, a):
    return {1: lambda: a(0, 0) + a(1, 1), 2: lambda: a(1, 0) + a(1, 1), 3: lambda: a(0, 0), 4: lambda: a(1, 1),
            5: lambda: a(0, 0) + a(0, 1), 6: lambda: a(1, 0) - a(0, 0), 7: lambda: a(0, 1) - a(1, 1)}[i]()


def _right(i, b):
    return {1: lambda: b(0, 0) + b(1, 1), 2: lambda: b(0, 0), 3: lambda: b(0, 1) - b(1, 1),
            4: lambda: b(1, 0) - b(0, 0), 5: lambda: b(1, 1), 6: lambda: b(0, 0) + b(0, 1),
            7: lambda: b(1, 0) + b(1, 1)}[i]()


def _strassen(product, base, emit):
    m5 = product(5)
    m3 = product(3)
    emit(0, 1, base(0, 1) + m5 + m3)
    m4 = product(4)
    c11 = base(0, 0) + m4 - m5
    m2 = product(2)
    emit(1, 0, base(1, 0) + m2 + m4)
    c22 = base(1, 1) + m3 - m2
    m1 = product(1)
    c11, c22 = c11 + m1, c22 + m1
    emit(0, 0, c11 + product(7))
    emit(1, 1, c22 + product(6))


def _vpu_jobs():
    blocks = [(u, j, r) for u, j in PASSES for r in range(KC - VPU_KEYS[u][j], KC, 16)]
    jobs = {}
    for n, block in enumerate(blocks):
        at = VPU_FIRST + (len(PASSES) - 1 + VPU_LAST - VPU_FIRST) * n / (len(blocks) - 1) + 1e-6
        jobs.setdefault(min(int(at), len(PASSES) - 1), []).append((*block, at - VPU_LEAD + VPU_NUDGE[n]))
    return jobs


def _scratch_shapes():
    n_spread = sum(VPU_ANY)
    return dict(
        k_buf=pltpu.VMEM((NB + len(STRADDLE), S // 2, LANES), I32), sqk_buf=pltpu.VMEM((5, HD, D), BF16),
        k_raw=pltpu.VMEM((TM // 2, D), I32), wo_buf=pltpu.VMEM((D, D), BF16),
        kb_buf0=pltpu.VMEM((DH, n_spread, LANES), F32), ot_buf=pltpu.VMEM((H, VR, S), F32),
        kx_buf=pltpu.VMEM((H // 2, NP * VPU_MAX, LANES), F32), s1_buf=pltpu.VMEM((5, HD, HF), BF16),
        kb_buf1=pltpu.VMEM((DH, n_spread, LANES), F32), h_buf=pltpu.VMEM((TM, D), F32),
        sv_buf=pltpu.VMEM((5, HD, HD), BF16), k_cur0=pltpu.VMEM((S // 2, LANES), I32),
        vt_buf=pltpu.VMEM((H, VR, S), F32), qt_buf=pltpu.VMEM((H, VR, S), F32), w1_buf=pltpu.VMEM((D, F), BF16),
        s2_buf=pltpu.VMEM((5, HF, HD), BF16), q_cur1=pltpu.VMEM((VR, S), F32), p_buf=pltpu.VMEM((NU, S, NQ), F32),
        out_buf=pltpu.VMEM((S, D), BF16), q_cur0=pltpu.VMEM((VR, S), F32), x_buf=pltpu.VMEM((S, D), BF16),
        b1_buf=pltpu.VMEM((F,), BF16), b2_buf=pltpu.VMEM((D,), BF16),
        sems=pltpu.SemaphoreType.DMA((2 * N_CHUNKS + 11,)), range_buf=pltpu.VMEM((2, 8, NQ), F32),
        xs_buf=pltpu.VMEM((5, HM, HD), BF16), so_buf=pltpu.VMEM((5, HD, HD), BF16),
        k_cur1=pltpu.VMEM((S // 2, LANES), I32), v_cur0=pltpu.VMEM((VR, S), F32),
        wqkv_buf=pltpu.VMEM((3, D, D), BF16), xn_buf=pltpu.VMEM((TM, D), BF16), v_cur1=pltpu.VMEM((VR, S), F32),
        w2_buf=pltpu.VMEM((F, D), BF16), s_buf=pltpu.VMEM((S, NQ), F32))


def _kernel(x_hbm, wqkv_hbm, wo_hbm, w1_hbm, b1_hbm, w2_hbm, b2_hbm, out_hbm,
            k_buf, sqk_buf, k_raw, wo_buf, kb_buf0, ot_buf, kx_buf, s1_buf, kb_buf1, h_buf, sv_buf, k_cur0,
            vt_buf, qt_buf, w1_buf, s2_buf, q_cur1, p_buf, out_buf, q_cur0, x_buf, b1_buf, b2_buf, sems,
            range_buf, xs_buf, so_buf, k_cur1, v_cur0, wqkv_buf, xn_buf, v_cur1, w2_buf, s_buf):
    q_cur, k_cur, v_cur, kb_buf = (q_cur0, q_cur1), (k_cur0, k_cur1), (v_cur0, v_cur1), (kb_buf0, kb_buf1)

    def x_copy(c):
        return pltpu.make_async_copy(x_hbm.at[0, _rows(c, TM)], x_buf.at[_rows(c, TM)], sems.at[c])

    def out_copy(c):
        return pltpu.make_async_copy(out_buf.at[_rows(c, TM)], out_hbm.at[0, _rows(c, TM)], sems.at[N_CHUNKS + c])

    copies = [(wqkv_hbm.at[:, pl.ds(j * D, D)], wqkv_buf.at[j]) for j in range(3)]
    copies += [(wo_hbm, wo_buf), (w1_hbm, w1_buf), (b1_hbm, b1_buf), (w2_hbm, w2_buf), (b2_hbm, b2_buf)]
    copies += [(out_buf.at[rows, cols], out_hbm.at[0, rows, cols]) for rows, cols in [
        (pl.ds(S - TM, HM), pl.ds(HD, D - HD)), (pl.ds(S - HM, HM), pl.ds(0, HD)),
        (pl.ds(S - TM, HM), pl.ds(0, HD)), (pl.ds(S - HM, HM), pl.ds(HD, D - HD))]]
    copies = [pltpu.make_async_copy(src, dst, sems.at[2 * N_CHUNKS - 1 + n]) for n, (src, dst) in enumerate(copies)]
    (wq_copy, wk_copy, wv_copy), tail_copies, last_copies = copies[:3], copies[3:8], copies[8:]

    def qk_block(r, c):
        return wqkv_buf.at[c, r * HD:(r + 1) * HD, :]

    def v_block(r, c):
        return wqkv_buf.at[2, r * HD:(r + 1) * HD, c * HD:(c + 1) * HD]

    def wo_block(r, c):
        return wo_buf.at[r * HD:(r + 1) * HD, c * HD:(c + 1) * HD]

    def w1_block(r, c):
        return w1_buf.at[r * HD:(r + 1) * HD, c * HF:(c + 1) * HF]

    def w2_block(r, c):
        return w2_buf.at[r * HF:(r + 1) * HF, c * HD:(c + 1) * HD]

    def weight_sums(dst, block):
        _, n_rows, n_cols = dst.shape

        def job(r, t):
            rows, cols = slice(r, r + 16), slice(t, min(t + HD, n_cols))

            def run(never, earlier):
                b = {(i, j): block(i, j).at[rows, cols][...].astype(F32) for i in range(2) for j in range(2)}
                for i in range(2):
                    reps = b[i, i].shape[1] // LANES
                    b[i, i] = _after(never, jnp.concatenate([earlier[0:16, 0:LANES]] * reps, axis=1), b[i, i])
                for i in B_SUMS:
                    dst[B_SUMS.index(i), rows, cols] = _right(i, lambda y, z: b[y, z]).astype(BF16)
            return run

        return [job(r, t) for r in range(0, n_rows, 16) for t in range(0, n_cols, HD)]

    def weights(i, sums, block):
        return sums[B_SUMS.index(i)] if i in B_SUMS else _right(i, block)[...]

    def normed(i):
        if i in A_SUMS:
            return xs_buf[A_SUMS.index(i)]
        return _left(i, lambda r, c: xn_buf[r * HM:(r + 1) * HM, c * HD:(c + 1) * HD])

    def norm_rows(load, r, sums=A_SUMS):
        halves = [_layernorm(load(half * HM + r)) for half in range(2)]
        out = [(xn_buf.at[pl.ds(half * HM + r, LN_ROWS)], halves[half].astype(BF16)) for half in range(2)]
        for i in sums:
            out.append((xs_buf.at[A_SUMS.index(i), pl.ds(r, LN_ROWS)],
                        _left(i, lambda a, b: halves[a][:, b * HD:(b + 1) * HD]).astype(BF16)))
        return out

    def flush(writes):
        for ref, val in writes:
            ref[...] = val

    def x_rows(c, never=None, earlier=None):
        def load(r):
            v = x_buf[pl.ds(pl.multiple_of(c * TM + r, LN_ROWS), LN_ROWS), :].astype(F32)
            if earlier is not None:
                v = jnp.concatenate([_after(never, earlier, v[:, :LANES]), v[:, LANES:]], axis=1)
            return v
        return load

    def key_block(p):
        b = 2 * DH * p // LANES
        for n, straddling in enumerate(STRADDLE):
            if isinstance(p, int):
                b = NB + n if p == straddling else b
            else:
                b = jnp.where(p == straddling, NB + n, b)
        return b

    def rotate_pair(keys, p):
        shift = (LANES - 2 * DH * p % LANES) % LANES
        return keys if isinstance(shift, int) and shift == 0 else pltpu.roll(keys, shift, 1)

    def put_keys(c, half, k_words):
        upper = lax.broadcasted_iota(I32, (HM // 2, LANES), 1) >= LANES // 2
        blocks = [k_words[:, b * LANES:(b + 1) * LANES] for b in range(NB)]
        blocks += [jnp.where(upper, blocks[2 * DH * p // LANES], blocks[2 * DH * p // LANES + 1]) for p in STRADDLE]
        for b, block in enumerate(blocks):
            k_buf[b, _rows(2 * c + half, HM // 2), :] = block
            ends = jnp.concatenate(
                [block[((j + 1) * KC - VPU_MAX) // 2:(j + 1) * KC // 2] for j in range(HM // KC)], axis=0)
            for p in range(H // 2):
                if key_block(p) == b:
                    kx_buf[p, _rows(2 * c + half, VPU_MAX * HM // KC), :] = _from_words(rotate_pair(ends, p)).astype(F32)

    def put_values(c, half, *v):
        rows = _rows(2 * c + half, HM)
        sub = lax.broadcasted_iota(I32, (8, HM), 0)
        vt = jnp.concatenate([part.astype(BF16).astype(F32).T for part in v], axis=0)
        for h in range(H):
            r0 = h * DH // 8 * 8
            if h % 2 == 0:
                vt_buf[h, 0:16, rows] = vt[r0:r0 + 16]
                vt_buf[h, 16:24, rows] = jnp.where(sub < 4, vt[r0 + 16:r0 + 24], 1.0)
            else:
                vt_buf[h, 0:8, rows] = jnp.where(sub < 4, 1.0, vt[r0:r0 + 8])
                vt_buf[h, 8:24, rows] = vt[r0 + 8:r0 + 24]

    def put_queries(c, half, q):
        qt = (q * QSCALE).T
        for h in range(H):
            qt_buf[h, :, _rows(2 * c + half, HM)] = jnp.concatenate(
                [qt[h * DH:(h + 1) * DH], jnp.zeros((VR - DH, HM), F32)], axis=0)

    x_copy(0).start()
    wk_copy.start()
    x_copy(0).wait()
    for r in range(0, HM, LN_ROWS):
        flush(norm_rows(x_rows(0), r, sums=()))
    wk_copy.wait()
    for cp in (wq_copy, wv_copy, x_copy(1)):
        cp.start()

    off = jnp.max(jnp.square(xn_buf[0:16, 0:LANES].astype(F32))) < 0.0
    k_raw[...] = _to_words(_mm(xn_buf[...], wqkv_buf[1]))
    wq_copy.wait()
    for c in range(2, N_CHUNKS):
        x_copy(c).start()
    q = _mm(xn_buf[...], wqkv_buf[0])
    h_buf[...] = q
    for half in range(2):
        put_keys(0, half, k_raw[half * HM // 2:(half + 1) * HM // 2, :])
    for n, job in enumerate(weight_sums(sqk_buf, qk_block)):
        job(off, q[n * SUM_ROW_STEP % (TM - 16) // 8 * 8:, n * NB // 48 * LANES:])
    wv_copy.wait()
    x_copy(1).wait()
    v = _mm(xn_buf[...], wqkv_buf[2])
    for half in range(2):
        put_queries(0, half, h_buf[half * HM:(half + 1) * HM, :])
    for n, job in enumerate(weight_sums(sv_buf, v_block)):
        job(off, v[n * SUM_ROW_STEP % (TM - 16) // 8 * 8:, n * NB // 16 * LANES:])
    writes = []
    for r in range(0, HM, LN_ROWS):
        writes += norm_rows(x_rows(1), r)
    for half in range(2):
        put_values(0, half, v[half * HM:(half + 1) * HM])
    flush(writes)
    for c in range(2, N_CHUNKS):
        x_copy(c).wait()
    for cp in tail_copies:
        cp.start()

    def qkv_chunk(c, carry):
        never = c < 0
        c_next = jnp.minimum(c + 1, N_CHUNKS - 1)
        todo, counts, writes = list(range(0, HM, LN_ROWS)), list(LN_PLAN), []

        def normalize_after(m):
            for k in range(counts.pop(0)):
                r, t = LN_ROW + k * LN_ROW_STEP, k * LN_LANE_STEP * LANES % m.shape[1]
                writes.extend(norm_rows(x_rows(c_next, never, m[r:r + LN_ROWS, t:t + LANES]), todo.pop(0)))
            return m

        v = {}
        rest = normalize_after(_mm(xn_buf[:, 2 * HD:], wqkv_buf[2, 2 * HD:, :2 * HD]))
        _strassen(lambda i: normalize_after(_mm(normed(i), weights(i, sv_buf, v_block))),
                  lambda r, col: rest[r * HM:(r + 1) * HM, col * HD:(col + 1) * HD],
                  lambda r, col, val: v.update({(r, col): val}))
        rest = normalize_after(_mm(
            xn_buf[:, 2 * HD:], jnp.concatenate([wqkv_buf[0, 2 * HD:, :], wqkv_buf[1, 2 * HD:, :]], axis=1)))
        _strassen(lambda i: normalize_after(_mm(normed(i), weights(i, sqk_buf, qk_block))),
                  lambda r, col: rest[r * HM:(r + 1) * HM, col * D:(col + 1) * D],
                  lambda r, col, val: put_keys(c, r, _to_words(val)) if col else put_queries(c, r, val))
        last = _mm(xn_buf[...], wqkv_buf[2, :, 2 * HD:])
        for r in range(2):
            put_values(c, r, v[r, 0], v[r, 1], last[r * HM:(r + 1) * HM])
        assert not todo
        flush(writes)
        return carry

    lax.fori_loop(1, N_CHUNKS, qkv_chunk, 0)

    vpu_jobs = _vpu_jobs()

    def spread_keys(side, pair, j):
        n = sum(VPU_ANY[:j])
        keys = kx_buf[pair, (j + 1) * VPU_MAX - VPU_ANY[j]:(j + 1) * VPU_MAX, :]
        for d in range(DH):
            kb_buf[side][d, n:n + VPU_ANY[j], :] = jnp.broadcast_to(
                keys[:, side * DH + d:side * DH + d + 1], (VPU_ANY[j], LANES))

    def attend(h, side, score=True, after_first_unit=None):
        scores, waiting = [], {}
        lo = hi = None
        if score:
            h_next = jnp.minimum(h + 1, H - 1)
            never = h < 0
        for g, (u, j) in enumerate(PASSES):
            cols, keys = slice(u * NQ, (u + 1) * NQ), slice(j * KC, (j + 1) * KC)
            n = KC - VPU_KEYS[u][j]
            if score:
                if j == 0:
                    qt = q_cur[side][:, cols].astype(BF16)
                s = _mm(_from_words(k_cur[side][j * KC // 2:(j * KC + n) // 2, :])[:, :VR], qt)
                scores.append(s)
                if u == (j + KEY_TURN) % NU:
                    used = slice(j * KC // 2, ((j + 1) * KC - min(n_vpu[j] for n_vpu in VPU_KEYS)) // 2)
                    if side:
                        k_cur[0][used, :] = rotate_pair(k_buf[key_block(h_next // 2), used, :], h_next // 2)
                    else:
                        k_cur[1][used, :] = pltpu.roll(k_cur[0][used, :], LANES - DH, 1)
                if j == QUERY_PASS:
                    q_cur[1 - side][:, cols] = qt_buf[h_next, :, cols]
            pv = _mm(v_cur[side][:, keys], p_buf[u, keys, :])
            acc = pv if j == 0 else acc + pv
            if score and u == (j + VALUE_TURN) % NU:
                v_cur[1 - side][:, keys] = vt_buf[h, :, keys]
            flush(waiting.pop(g, []))
            if j == NP - 1:
                ot_buf[h - 1, :, cols] = acc
                top = jnp.maximum(jnp.maximum(jnp.abs(acc[0:8]), jnp.abs(acc[8:16])), jnp.abs(acc[16:24]))
                sub = lax.broadcasted_iota(I32, (8, NQ), 0)
                total = jnp.where(sub >= 4, acc[16:24], ACC_MAX) if side else jnp.where(sub < 4, acc[0:8], ACC_MAX)
                lo = total if lo is None else jnp.minimum(lo, total)
                hi = top if hi is None else jnp.maximum(hi, top)
            if g == NP + 10 and after_first_unit:
                after_first_unit()
            if not score:
                continue
            for uu, jj, r, time in vpu_jobs.get(g, []):
                first = sum(VPU_ANY[:jj]) + r - (KC - VPU_ANY[jj])
                val = None
                for d in range(DH):
                    kb = kb_buf[side][d, first:first + 16, :]
                    when = time + (d - VPU_PACED[0]) / DH * VPU_SPAN
                    if d in VPU_PACED and when >= 0:
                        earlier = scores[min(int(when), g)]
                        row = int(when % 1 * (earlier.shape[0] - 8)) // 8 * 8
                        kb = _after(never, earlier[row:row + 16, VPU_LANE:VPU_LANE + LANES], kb)
                    term = jnp.concatenate(
                        [kb * q_cur[side][d:d + 1, t:t + LANES] for t in range(uu * NQ, (uu + 1) * NQ, LANES)], axis=1)
                    val = term if val is None else val + term
                write = (p_buf.at[uu, jj * KC + r:jj * KC + r + 16, :], jnp.exp2(val))
                if PASSES.index((uu, jj)) <= g:
                    flush([write])
                else:
                    waiting.setdefault(PASSES.index((uu, jj)), []).append(write)
            p_buf[u, j * KC:j * KC + n, :] = jnp.exp2(s)
            ahead = (j + SPREAD_AHEAD) % NP
            if (ahead + SPREAD_TURN) % NU == u:
                spread_keys(1 - side, h_next // 2, ahead)
        assert not waiting
        range_buf[0] = jnp.minimum(range_buf[0], lo)
        range_buf[1] = jnp.maximum(range_buf[1], hi)

    def attend_shifted(i, carry):
        h, cols = i // NU, _rows(i % NU, NQ)
        qt = qt_buf[h, :, cols].astype(BF16)

        def score(j, m):
            keys = pltpu.roll(k_buf[key_block(h // 2), _rows(j, KC // 2), :], (LANES - h * DH % LANES) % LANES, 1)
            s = _mm(_from_words(keys)[:, :VR], qt)
            s_buf[_rows(j, KC), :] = s
            return jnp.maximum(m, jnp.max(s.reshape(KC // 8, 8, NQ), axis=0))

        m = lax.fori_loop(0, NP, score, jnp.full((8, NQ), -jnp.inf, F32))
        m = jnp.max(m, axis=0, keepdims=True)

        def weigh(j, acc):
            return acc + _mm(vt_buf[h, :, _rows(j, KC)], jnp.exp2(s_buf[_rows(j, KC), :] - m))

        ot_buf[h, :, cols] = lax.fori_loop(0, NP, weigh, jnp.zeros((VR, NQ), F32))
        return carry

    for cp in tail_copies:
        cp.wait()
    off = jnp.max(jnp.square(qt_buf[0, 0:8, 0:LANES])) < 0.0
    jobs = weight_sums(so_buf, wo_block) + weight_sums(s1_buf, w1_block) + weight_sums(s2_buf, w2_block)
    n_jobs = len(jobs)
    for g, (u, j) in enumerate(PASSES):
        if j == 0:
            qt = qt_buf[0, :, u * NQ:(u + 1) * NQ].astype(BF16)
        s = _mm(_from_words(k_buf[0, j * KC // 2:(j + 1) * KC // 2, :])[:, :VR], qt)
        p_buf[u, j * KC:(j + 1) * KC, :] = jnp.exp2(s)
        while jobs and len(jobs) > n_jobs * (1 - (g + 3) / len(PASSES)):
            jobs.pop(0)(off, s[len(jobs) % 2 * 96:])
    for j in range(NP):
        spread_keys(1, 0, j)
    k_cur[1][...] = pltpu.roll(k_buf[0], LANES - DH, 1)
    q_cur[1][...] = qt_buf[1]
    v_cur[1][...] = vt_buf[0]
    range_buf[0] = jnp.full((8, NQ), ACC_MAX, F32)
    range_buf[1] = jnp.zeros((8, NQ), F32)

    def head(h, carry):
        lax.cond(h % 2 == 1, lambda: attend(h, 1), lambda: attend(h, 0))
        return carry

    lax.fori_loop(1, H, head, None)

    def attention_out(c, n):
        rows = _rows(c, n)
        sub = lax.broadcasted_iota(I32, (8, n), 0)
        parts = []
        for h in range(0, H, 2):
            even, odd = ot_buf[h, :, rows], ot_buf[h + 1, :, rows]
            even = even * (1.0 / even[VR - 1:VR])
            odd = odd * (1.0 / odd[0:1])
            parts += [even[0:16], jnp.where(sub < 4, even[16:24], odd[0:8]), odd[8:24]]
        return jnp.concatenate(parts, axis=0).T

    def project(c):
        o = attention_out(c, TM)
        x = x_buf[_rows(c, TM), :].astype(F32)
        rest = x[:, :2 * HD] + _mm(o[:, 2 * HD:].astype(BF16), wo_buf[2 * HD:, :2 * HD])
        last = x[:, 2 * HD:] + _mm(o.astype(BF16), wo_buf[:, 2 * HD:])
        h = {}
        _strassen(lambda i: _mm(_left(i, lambda r, col: o[r * HM:(r + 1) * HM, col * HD:(col + 1) * HD]).astype(BF16),
                                weights(i, so_buf, wo_block)),
                  lambda r, col: rest[r * HM:(r + 1) * HM, col * HD:(col + 1) * HD],
                  lambda r, col, val: h.update({(r, col): val}))
        return jnp.concatenate(
            [jnp.concatenate([h[r, 0], h[r, 1], last[r * HM:(r + 1) * HM]], axis=1) for r in range(2)], axis=0)

    def ffn(c, is_last):
        act = {}

        def activate(r, col, f):
            f = jnp.where(f > 0.0, f, 0.0)
            act[r, col] = f * f

        rest = _mm(xn_buf[:, 2 * HD:], w1_buf[2 * HD:, :]) + b1_buf[...].astype(F32)[None, :]
        _strassen(lambda i: _mm(normed(i), weights(i, s1_buf, w1_block)),
                  lambda r, col: rest[r * HM:(r + 1) * HM, col * HF:(col + 1) * HF], activate)
        todo, writes = [], []
        if not is_last:
            h_next = project(c + 1)
            todo = list(range(0, HM, LN_ROWS))
        b2 = b2_buf[...].astype(F32)[None, :]
        early = [_mm(act[r, 1 - r].astype(BF16), w2_buf[(1 - r) * HF:(2 - r) * HF, 2 * HD:]) for r in range(2)]
        for r in range(2):
            last = early[r] + _mm(act[r, r].astype(BF16), w2_buf[r * HF:(r + 1) * HF, 2 * HD:])
            out_buf[_rows(2 * c + r, HM), 2 * HD:] = (
                h_buf[r * HM:(r + 1) * HM, 2 * HD:] + b2[:, 2 * HD:] + last).astype(BF16)

        def product(i):
            m = _mm(_left(i, lambda r, col: act[r, col]).astype(BF16), weights(i, s2_buf, w2_block))

            def load(r):
                v = h_next[r:r + LN_ROWS]
                return jnp.concatenate([_after(c < 0, m[:LN_ROWS, :LANES], v[:, :LANES]), v[:, LANES:]], axis=1)

            for _ in range(3):
                if todo:
                    writes.extend(norm_rows(load, todo.pop(0)))
            return m

        def put_out(r, col, val):
            out_buf[_rows(2 * c + r, HM), col * HD:(col + 1) * HD] = val.astype(BF16)
            if is_last and (r, col) == (1, 0):
                for cp in last_copies[:2]:
                    cp.start()

        _strassen(product,
                  lambda r, col: h_buf[r * HM:(r + 1) * HM, col * HD:(col + 1) * HD] + b2[:, col * HD:(col + 1) * HD],
                  put_out)
        assert not todo
        if not is_last:
            h_buf[...] = h_next
            flush(writes)

    h_first = []
    attend(H, 0, score=False, after_first_unit=lambda: h_first.append(project(0)))
    h_buf[...] = h_first[0]
    writes = []
    for r in range(0, HM, LN_ROWS):
        writes += norm_rows(lambda r0: h_first[0][r0:r0 + LN_ROWS], r)
    flush(writes)
    safe = jnp.logical_and(range_buf[0] >= SUM_MIN, range_buf[1] <= ACC_MAX)

    @pl.when(jnp.max(jnp.where(safe, 0.0, 1.0)) > 0.0)
    def _():
        lax.fori_loop(0, H * NU, attend_shifted, 0)

        def project_again(i, carry):
            rows = _rows(i, LANES)
            h_buf[rows, :] = x_buf[rows, :].astype(F32) + _mm(attention_out(i, LANES).astype(BF16), wo_buf[...])
            return carry

        def normalize_again(i, carry):
            flush(norm_rows(lambda r: h_buf[pl.ds(r, LN_ROWS), :], pl.multiple_of(i * LN_ROWS, LN_ROWS)))
            return carry

        lax.fori_loop(0, TM // LANES, project_again, 0)
        lax.fori_loop(0, HM // LN_ROWS, normalize_again, 0)

    def ffn_chunk(c, carry):
        ffn(c, False)
        out_copy(c).start()
        return carry

    lax.fori_loop(0, N_CHUNKS - 1, ffn_chunk, 0)
    ffn(N_CHUNKS - 1, True)
    for cp in last_copies[2:]:
        cp.start()
    for cp in [out_copy(c) for c in range(N_CHUNKS - 1)] + last_copies:
        cp.wait()


@jax.jit
def pallas_sequential_preLN__softmax_full_mha__dense_activation_squared_relu__prompt_kernel(
    A_x: jax.Array,
    A_wqkv: jax.Array,
    A_wo: jax.Array,
    B_x: jax.Array,
    B_w1: jax.Array,
    B_b1: jax.Array,
    B_w2: jax.Array,
    B_b2: jax.Array,
):
    del B_x
    any_spec = pl.BlockSpec(memory_space=pl.ANY)
    return pl.pallas_call(
        _kernel,
        out_shape=jax.ShapeDtypeStruct(A_x.shape, A_x.dtype),
        in_specs=[any_spec] * 7,
        out_specs=any_spec,
        scratch_shapes=list(_scratch_shapes().values()),
        compiler_params=pltpu.CompilerParams(
            vmem_limit_bytes=110 * 2**20,
            flags={"XLA_TPU_EVENLY_DISTRIBUTE_CRITICAL_NODES": True}),
    )(A_x, A_wqkv, A_wo, B_w1, B_b1, B_w2, B_b2)
```

```python
import jax
import jax.numpy as jnp
import numpy as np
from jax import lax
import jax.experimental.pallas as pl
import jax.experimental.pallas.tpu as pltpu


F32, BF16, I32 = jnp.float32, jnp.bfloat16, jnp.int32
S, D, H, DH, F = 2048, 640, 32, 20, 1536
EPS = 1e-5
QSCALE = float(DH ** -0.5 * np.log2(np.e))
SUM_MIN = 2.0 ** -60
ACC_MAX = 2.0 ** 100

LANES = 128
NB = D // LANES
TM = 512
N_CHUNKS = S // TM
HM = TM // 2
HD = 2 * LANES
HF = F // 2
LN_ROWS = 16
NQ = 512
NU = S // NQ
KC = 128
NP = S // KC
VR = 24
STRADDLE = [p for p in range(H // 2) if 2 * DH * p % LANES + 2 * DH > LANES]

VPU_KEYS = [[16 * int(x[j % len(x)]) for j in range(NP)]
            for x in "0011111211111112/11111112/11111112/11111112".split("/")]
VPU_ANY = [max(n[j] for n in VPU_KEYS) for j in range(NP)]
VPU_MAX = max(VPU_ANY)
PASSES = [(u, j) for u in range(NU) for j in range(NP)]

VPU_FIRST, VPU_LAST = 1.0, 0.0
VPU_LEAD, VPU_SPAN = 0.77, 0.9
VPU_NUDGE = [(ord(ch) - ord("m")) / 20 for ch in
             "immjkmmmmllmnkkmmmmopmknmmmmmmmmnlmmmmmklmommmmmmmmmmjmjmlmmjmmmnmmmom"]
VPU_PACED = range(1, DH, 6)
VPU_LANE = 256
KEY_TURN, VALUE_TURN, QUERY_PASS = 2, 1, 9
SPREAD_TURN, SPREAD_AHEAD = 2, 5
LN_PLAN = [int(n) for n in "0010101021212122"]
LN_ROW, LN_ROW_STEP, LN_LANE_STEP = 32, 64, 3
SUM_ROW_STEP = 56

A_SUMS = (1, 2, 5, 6, 7)
B_SUMS = (1, 3, 4, 6, 7)


def _mm(a, b):
    return jnp.dot(a, b, preferred_element_type=F32)


def _after(never, earlier, value):
    return jnp.where(never, earlier, value)


def _layernorm(v):
    mean = jnp.sum(v, axis=-1, keepdims=True) * (1.0 / D)
    c = v - mean
    var = jnp.sum(c * c, axis=-1, keepdims=True) * (1.0 / D)
    return c * lax.rsqrt(var + EPS)


def _rows(i, n):
    return pl.ds(i * n, n) if isinstance(i, int) else pl.ds(pl.multiple_of(i * n, n), n)


def _to_words(v):
    return pltpu.bitcast(v.astype(BF16), I32)


def _from_words(w):
    return pltpu.bitcast(w, BF16)


def _left(i, a):
    return {1: lambda: a(0, 0) + a(1, 1), 2: lambda: a(1, 0) + a(1, 1), 3: lambda: a(0, 0), 4: lambda: a(1, 1),
            5: lambda: a(0, 0) + a(0, 1), 6: lambda: a(1, 0) - a(0, 0), 7: lambda: a(0, 1) - a(1, 1)}[i]()


def _right(i, b):
    return {1: lambda: b(0, 0) + b(1, 1), 2: lambda: b(0, 0), 3: lambda: b(0, 1) - b(1, 1),
            4: lambda: b(1, 0) - b(0, 0), 5: lambda: b(1, 1), 6: lambda: b(0, 0) + b(0, 1),
            7: lambda: b(1, 0) + b(1, 1)}[i]()


def _strassen(product, base, emit):
    m5 = product(5)
    m3 = product(3)
    emit(0, 1, base(0, 1) + m5 + m3)
    m4 = product(4)
    c11 = base(0, 0) + m4 - m5
    m2 = product(2)
    emit(1, 0, base(1, 0) + m2 + m4)
    c22 = base(1, 1) + m3 - m2
    m1 = product(1)
    c11, c22 = c11 + m1, c22 + m1
    emit(0, 0, c11 + product(7))
    emit(1, 1, c22 + product(6))


def _vpu_jobs():
    blocks = [(u, j, r) for u, j in PASSES for r in range(KC - VPU_KEYS[u][j], KC, 16)]
    jobs = {}
    for n, block in enumerate(blocks):
        at = VPU_FIRST + (len(PASSES) - 1 + VPU_LAST - VPU_FIRST) * n / (len(blocks) - 1) + 1e-6
        jobs.setdefault(min(int(at), len(PASSES) - 1), []).append((*block, at - VPU_LEAD + VPU_NUDGE[n]))
    return jobs


def _scratch_shapes():
    n_spread = sum(VPU_ANY)
    return dict(
        k_buf=pltpu.VMEM((NB + len(STRADDLE), S // 2, LANES), I32), sqk_buf=pltpu.VMEM((5, HD, D), BF16),
        k_raw=pltpu.VMEM((TM // 2, D), I32), wo_buf=pltpu.VMEM((D, D), BF16),
        kb_buf0=pltpu.VMEM((DH, n_spread, LANES), F32), ot_buf=pltpu.VMEM((H, VR, S), F32),
        kx_buf=pltpu.VMEM((H // 2, NP * VPU_MAX, LANES), F32), s1_buf=pltpu.VMEM((5, HD, HF), BF16),
        kb_buf1=pltpu.VMEM((DH, n_spread, LANES), F32), h_buf=pltpu.VMEM((TM, D), F32),
        sv_buf=pltpu.VMEM((5, HD, HD), BF16), k_cur0=pltpu.VMEM((S // 2, LANES), I32),
        vt_buf=pltpu.VMEM((H, VR, S), F32), qt_buf=pltpu.VMEM((H, VR, S), F32), w1_buf=pltpu.VMEM((D, F), BF16),
        s2_buf=pltpu.VMEM((5, HF, HD), BF16), q_cur1=pltpu.VMEM((VR, S), F32), p_buf=pltpu.VMEM((NU, S, NQ), F32),
        out_buf=pltpu.VMEM((S, D), BF16), q_cur0=pltpu.VMEM((VR, S), F32), x_buf=pltpu.VMEM((S, D), BF16),
        b1_buf=pltpu.VMEM((F,), BF16), b2_buf=pltpu.VMEM((D,), BF16),
        sems=pltpu.SemaphoreType.DMA((2 * N_CHUNKS + 12,)), range_buf=pltpu.VMEM((2, 8, NQ), F32),
        xs_buf=pltpu.VMEM((5, HM, HD), BF16), so_buf=pltpu.VMEM((5, HD, HD), BF16),
        k_cur1=pltpu.VMEM((S // 2, LANES), I32), v_cur0=pltpu.VMEM((VR, S), F32),
        wqkv_buf=pltpu.VMEM((3, D, D), BF16), xn_buf=pltpu.VMEM((TM, D), BF16), v_cur1=pltpu.VMEM((VR, S), F32),
        w2_buf=pltpu.VMEM((F, D), BF16), s_buf=pltpu.VMEM((S, NQ), F32))


def _kernel(x_hbm, wqkv_hbm, wo_hbm, w1_hbm, b1_hbm, w2_hbm, b2_hbm, out_hbm,
            k_buf, sqk_buf, k_raw, wo_buf, kb_buf0, ot_buf, kx_buf, s1_buf, kb_buf1, h_buf, sv_buf, k_cur0,
            vt_buf, qt_buf, w1_buf, s2_buf, q_cur1, p_buf, out_buf, q_cur0, x_buf, b1_buf, b2_buf, sems,
            range_buf, xs_buf, so_buf, k_cur1, v_cur0, wqkv_buf, xn_buf, v_cur1, w2_buf, s_buf):
    q_cur, k_cur, v_cur, kb_buf = (q_cur0, q_cur1), (k_cur0, k_cur1), (v_cur0, v_cur1), (kb_buf0, kb_buf1)

    def x_copy(c):
        return pltpu.make_async_copy(x_hbm.at[0, _rows(c, TM)], x_buf.at[_rows(c, TM)], sems.at[c])

    def out_copy(c):
        return pltpu.make_async_copy(out_buf.at[_rows(c, TM)], out_hbm.at[0, _rows(c, TM)], sems.at[N_CHUNKS + c])

    copies = [(wqkv_hbm.at[:, pl.ds(j * D, D)], wqkv_buf.at[j]) for j in range(3)]
    copies += [(wo_hbm, wo_buf), (w1_hbm, w1_buf), (b1_hbm, b1_buf), (w2_hbm, w2_buf), (b2_hbm, b2_buf)]
    copies += [(out_buf.at[rows, cols], out_hbm.at[0, rows, cols]) for rows, cols in [
        (pl.ds(S - TM, HM), pl.ds(HD, D - HD)), (pl.ds(S - HM, HM), pl.ds(2 * HD, LANES)),
        (pl.ds(S - HM, HM), pl.ds(0, HD)), (pl.ds(S - TM, HM), pl.ds(0, HD)), (pl.ds(S - HM, HM), pl.ds(HD, HD))]]
    copies = [pltpu.make_async_copy(src, dst, sems.at[2 * N_CHUNKS - 1 + n]) for n, (src, dst) in enumerate(copies)]
    (wq_copy, wk_copy, wv_copy), tail_copies, last_copies = copies[:3], copies[3:8], copies[8:]

    def qk_block(r, c):
        return wqkv_buf.at[c, r * HD:(r + 1) * HD, :]

    def v_block(r, c):
        return wqkv_buf.at[2, r * HD:(r + 1) * HD, c * HD:(c + 1) * HD]

    def wo_block(r, c):
        return wo_buf.at[r * HD:(r + 1) * HD, c * HD:(c + 1) * HD]

    def w1_block(r, c):
        return w1_buf.at[r * HD:(r + 1) * HD, c * HF:(c + 1) * HF]

    def w2_block(r, c):
        return w2_buf.at[r * HF:(r + 1) * HF, c * HD:(c + 1) * HD]

    def weight_sums(dst, block):
        _, n_rows, n_cols = dst.shape

        def job(r, t):
            rows, cols = slice(r, r + 16), slice(t, min(t + HD, n_cols))

            def run(never, earlier):
                b = {(i, j): block(i, j).at[rows, cols][...].astype(F32) for i in range(2) for j in range(2)}
                for i in range(2):
                    reps = b[i, i].shape[1] // LANES
                    b[i, i] = _after(never, jnp.concatenate([earlier[0:16, 0:LANES]] * reps, axis=1), b[i, i])
                for i in B_SUMS:
                    dst[B_SUMS.index(i), rows, cols] = _right(i, lambda y, z: b[y, z]).astype(BF16)
            return run

        return [job(r, t) for r in range(0, n_rows, 16) for t in range(0, n_cols, HD)]

    def weights(i, sums, block):
        return sums[B_SUMS.index(i)] if i in B_SUMS else _right(i, block)[...]

    def normed(i):
        if i in A_SUMS:
            return xs_buf[A_SUMS.index(i)]
        return _left(i, lambda r, c: xn_buf[r * HM:(r + 1) * HM, c * HD:(c + 1) * HD])

    def norm_rows(load, r, sums=A_SUMS):
        halves = [_layernorm(load(half * HM + r)) for half in range(2)]
        out = [(xn_buf.at[pl.ds(half * HM + r, LN_ROWS)], halves[half].astype(BF16)) for half in range(2)]
        for i in sums:
            out.append((xs_buf.at[A_SUMS.index(i), pl.ds(r, LN_ROWS)],
                        _left(i, lambda a, b: halves[a][:, b * HD:(b + 1) * HD]).astype(BF16)))
        return out

    def flush(writes):
        for ref, val in writes:
            ref[...] = val

    def x_rows(c, never=None, earlier=None):
        def load(r):
            v = x_buf[pl.ds(pl.multiple_of(c * TM + r, LN_ROWS), LN_ROWS), :].astype(F32)
            if earlier is not None:
                v = jnp.concatenate([_after(never, earlier, v[:, :LANES]), v[:, LANES:]], axis=1)
            return v
        return load

    def key_block(p):
        b = 2 * DH * p // LANES
        for n, straddling in enumerate(STRADDLE):
            if isinstance(p, int):
                b = NB + n if p == straddling else b
            else:
                b = jnp.where(p == straddling, NB + n, b)
        return b

    def rotate_pair(keys, p):
        shift = (LANES - 2 * DH * p % LANES) % LANES
        return keys if isinstance(shift, int) and shift == 0 else pltpu.roll(keys, shift, 1)

    def put_keys(c, half, k_words):
        upper = lax.broadcasted_iota(I32, (HM // 2, LANES), 1) >= LANES // 2
        blocks = [k_words[:, b * LANES:(b + 1) * LANES] for b in range(NB)]
        blocks += [jnp.where(upper, blocks[2 * DH * p // LANES], blocks[2 * DH * p // LANES + 1]) for p in STRADDLE]
        for b, block in enumerate(blocks):
            k_buf[b, _rows(2 * c + half, HM // 2), :] = block
            ends = jnp.concatenate(
                [block[((j + 1) * KC - VPU_MAX) // 2:(j + 1) * KC // 2] for j in range(HM // KC)], axis=0)
            for p in range(H // 2):
                if key_block(p) == b:
                    kx_buf[p, _rows(2 * c + half, VPU_MAX * HM // KC), :] = _from_words(rotate_pair(ends, p)).astype(F32)

    def put_values(c, half, *v):
        rows = _rows(2 * c + half, HM)
        sub = lax.broadcasted_iota(I32, (8, HM), 0)
        vt = jnp.concatenate([part.astype(BF16).astype(F32).T for part in v], axis=0)
        for h in range(H):
            r0 = h * DH // 8 * 8
            if h % 2 == 0:
                vt_buf[h, 0:16, rows] = vt[r0:r0 + 16]
                vt_buf[h, 16:24, rows] = jnp.where(sub < 4, vt[r0 + 16:r0 + 24], 1.0)
            else:
                vt_buf[h, 0:8, rows] = jnp.where(sub < 4, 1.0, vt[r0:r0 + 8])
                vt_buf[h, 8:24, rows] = vt[r0 + 8:r0 + 24]

    def put_queries(c, half, q):
        qt = (q * QSCALE).T
        for h in range(H):
            qt_buf[h, :, _rows(2 * c + half, HM)] = jnp.concatenate(
                [qt[h * DH:(h + 1) * DH], jnp.zeros((VR - DH, HM), F32)], axis=0)

    x_copy(0).start()
    wk_copy.start()
    x_copy(0).wait()
    for r in range(0, HM, LN_ROWS):
        flush(norm_rows(x_rows(0), r, sums=()))
    wk_copy.wait()
    for cp in (wq_copy, wv_copy, x_copy(1)):
        cp.start()

    off = jnp.max(jnp.square(xn_buf[0:16, 0:LANES].astype(F32))) < 0.0
    k_raw[...] = _to_words(_mm(xn_buf[...], wqkv_buf[1]))
    wq_copy.wait()
    for c in range(2, N_CHUNKS):
        x_copy(c).start()
    q = _mm(xn_buf[...], wqkv_buf[0])
    h_buf[...] = q
    for half in range(2):
        put_keys(0, half, k_raw[half * HM // 2:(half + 1) * HM // 2, :])
    for n, job in enumerate(weight_sums(sqk_buf, qk_block)):
        job(off, q[n * SUM_ROW_STEP % (TM - 16) // 8 * 8:, n * NB // 48 * LANES:])
    wv_copy.wait()
    x_copy(1).wait()
    v = _mm(xn_buf[...], wqkv_buf[2])
    for half in range(2):
        put_queries(0, half, h_buf[half * HM:(half + 1) * HM, :])
    for n, job in enumerate(weight_sums(sv_buf, v_block)):
        job(off, v[n * SUM_ROW_STEP % (TM - 16) // 8 * 8:, n * NB // 16 * LANES:])
    writes = []
    for r in range(0, HM, LN_ROWS):
        writes += norm_rows(x_rows(1), r)
    for half in range(2):
        put_values(0, half, v[half * HM:(half + 1) * HM])
    flush(writes)
    for c in range(2, N_CHUNKS):
        x_copy(c).wait()
    for cp in tail_copies:
        cp.start()

    def qkv_chunk(c, carry):
        never = c < 0
        c_next = jnp.minimum(c + 1, N_CHUNKS - 1)
        todo, counts, writes = list(range(0, HM, LN_ROWS)), list(LN_PLAN), []

        def normalize_after(m):
            for k in range(counts.pop(0)):
                r, t = LN_ROW + k * LN_ROW_STEP, k * LN_LANE_STEP * LANES % m.shape[1]
                writes.extend(norm_rows(x_rows(c_next, never, m[r:r + LN_ROWS, t:t + LANES]), todo.pop(0)))
            return m

        v = {}
        rest = normalize_after(_mm(xn_buf[:, 2 * HD:], wqkv_buf[2, 2 * HD:, :2 * HD]))
        _strassen(lambda i: normalize_after(_mm(normed(i), weights(i, sv_buf, v_block))),
                  lambda r, col: rest[r * HM:(r + 1) * HM, col * HD:(col + 1) * HD],
                  lambda r, col, val: v.update({(r, col): val}))
        rest = normalize_after(_mm(
            xn_buf[:, 2 * HD:], jnp.concatenate([wqkv_buf[0, 2 * HD:, :], wqkv_buf[1, 2 * HD:, :]], axis=1)))
        _strassen(lambda i: normalize_after(_mm(normed(i), weights(i, sqk_buf, qk_block))),
                  lambda r, col: rest[r * HM:(r + 1) * HM, col * D:(col + 1) * D],
                  lambda r, col, val: put_keys(c, r, _to_words(val)) if col else put_queries(c, r, val))
        last = _mm(xn_buf[...], wqkv_buf[2, :, 2 * HD:])
        for r in range(2):
            put_values(c, r, v[r, 0], v[r, 1], last[r * HM:(r + 1) * HM])
        assert not todo
        flush(writes)
        return carry

    lax.fori_loop(1, N_CHUNKS, qkv_chunk, 0)

    vpu_jobs = _vpu_jobs()

    def spread_keys(side, pair, j):
        n = sum(VPU_ANY[:j])
        keys = kx_buf[pair, (j + 1) * VPU_MAX - VPU_ANY[j]:(j + 1) * VPU_MAX, :]
        for d in range(DH):
            kb_buf[side][d, n:n + VPU_ANY[j], :] = jnp.broadcast_to(
                keys[:, side * DH + d:side * DH + d + 1], (VPU_ANY[j], LANES))

    def attend(h, side, score=True, after_first_unit=None):
        scores, waiting = [], {}
        lo = hi = None
        if score:
            h_next = jnp.minimum(h + 1, H - 1)
            never = h < 0
        for g, (u, j) in enumerate(PASSES):
            cols, keys = slice(u * NQ, (u + 1) * NQ), slice(j * KC, (j + 1) * KC)
            n = KC - VPU_KEYS[u][j]
            if score:
                if j == 0:
                    qt = q_cur[side][:, cols].astype(BF16)
                s = _mm(_from_words(k_cur[side][j * KC // 2:(j * KC + n) // 2, :])[:, :VR], qt)
                scores.append(s)
                if u == (j + KEY_TURN) % NU:
                    used = slice(j * KC // 2, ((j + 1) * KC - min(n_vpu[j] for n_vpu in VPU_KEYS)) // 2)
                    if side:
                        k_cur[0][used, :] = rotate_pair(k_buf[key_block(h_next // 2), used, :], h_next // 2)
                    else:
                        k_cur[1][used, :] = pltpu.roll(k_cur[0][used, :], LANES - DH, 1)
                if j == QUERY_PASS:
                    q_cur[1 - side][:, cols] = qt_buf[h_next, :, cols]
            pv = _mm(v_cur[side][:, keys], p_buf[u, keys, :])
            acc = pv if j == 0 else acc + pv
            if score and u == (j + VALUE_TURN) % NU:
                v_cur[1 - side][:, keys] = vt_buf[h, :, keys]
            flush(waiting.pop(g, []))
            if j == NP - 1:
                ot_buf[h - 1, :, cols] = acc
                top = jnp.maximum(jnp.maximum(jnp.abs(acc[0:8]), jnp.abs(acc[8:16])), jnp.abs(acc[16:24]))
                sub = lax.broadcasted_iota(I32, (8, NQ), 0)
                total = jnp.where(sub >= 4, acc[16:24], ACC_MAX) if side else jnp.where(sub < 4, acc[0:8], ACC_MAX)
                lo = total if lo is None else jnp.minimum(lo, total)
                hi = top if hi is None else jnp.maximum(hi, top)
            if g == NP + 10 and after_first_unit:
                after_first_unit()
            if not score:
                continue
            for uu, jj, r, time in vpu_jobs.get(g, []):
                first = sum(VPU_ANY[:jj]) + r - (KC - VPU_ANY[jj])
                val = None
                for d in range(DH):
                    kb = kb_buf[side][d, first:first + 16, :]
                    when = time + (d - VPU_PACED[0]) / DH * VPU_SPAN
                    if d in VPU_PACED and when >= 0:
                        earlier = scores[min(int(when), g)]
                        row = int(when % 1 * (earlier.shape[0] - 8)) // 8 * 8
                        kb = _after(never, earlier[row:row + 16, VPU_LANE:VPU_LANE + LANES], kb)
                    term = jnp.concatenate(
                        [kb * q_cur[side][d:d + 1, t:t + LANES] for t in range(uu * NQ, (uu + 1) * NQ, LANES)], axis=1)
                    val = term if val is None else val + term
                write = (p_buf.at[uu, jj * KC + r:jj * KC + r + 16, :], jnp.exp2(val))
                if PASSES.index((uu, jj)) <= g:
                    flush([write])
                else:
                    waiting.setdefault(PASSES.index((uu, jj)), []).append(write)
            p_buf[u, j * KC:j * KC + n, :] = jnp.exp2(s)
            ahead = (j + SPREAD_AHEAD) % NP
            if (ahead + SPREAD_TURN) % NU == u:
                spread_keys(1 - side, h_next // 2, ahead)
        assert not waiting
        range_buf[0] = jnp.minimum(range_buf[0], lo)
        range_buf[1] = jnp.maximum(range_buf[1], hi)

    def attend_shifted(i, carry):
        h, cols = i // NU, _rows(i % NU, NQ)
        qt = qt_buf[h, :, cols].astype(BF16)

        def score(j, m):
            keys = pltpu.roll(k_buf[key_block(h // 2), _rows(j, KC // 2), :], (LANES - h * DH % LANES) % LANES, 1)
            s = _mm(_from_words(keys)[:, :VR], qt)
            s_buf[_rows(j, KC), :] = s
            return jnp.maximum(m, jnp.max(s.reshape(KC // 8, 8, NQ), axis=0))

        m = lax.fori_loop(0, NP, score, jnp.full((8, NQ), -jnp.inf, F32))
        m = jnp.max(m, axis=0, keepdims=True)

        def weigh(j, acc):
            return acc + _mm(vt_buf[h, :, _rows(j, KC)], jnp.exp2(s_buf[_rows(j, KC), :] - m))

        ot_buf[h, :, cols] = lax.fori_loop(0, NP, weigh, jnp.zeros((VR, NQ), F32))
        return carry

    for cp in tail_copies:
        cp.wait()
    jobs = weight_sums(so_buf, wo_block) + weight_sums(s1_buf, w1_block) + weight_sums(s2_buf, w2_block)
    n_jobs = len(jobs)
    for g, (u, j) in enumerate(PASSES):
        if j == 0:
            qt = qt_buf[0, :, u * NQ:(u + 1) * NQ].astype(BF16)
        s = _mm(_from_words(k_buf[0, j * KC // 2:(j + 1) * KC // 2, :])[:, :VR], qt)
        p_buf[u, j * KC:(j + 1) * KC, :] = jnp.exp2(s)
        while jobs and len(jobs) > n_jobs * (1 - (g + 3) / len(PASSES)):
            jobs.pop(0)(off, s[len(jobs) % 2 * 96:])
    for j in range(NP):
        spread_keys(1, 0, j)
    k_cur[1][...] = pltpu.roll(k_buf[0], LANES - DH, 1)
    q_cur[1][...] = qt_buf[1]
    v_cur[1][...] = vt_buf[0]
    range_buf[0] = jnp.full((8, NQ), ACC_MAX, F32)
    range_buf[1] = jnp.zeros((8, NQ), F32)

    def head(h, carry):
        lax.cond(h % 2 == 1, lambda: attend(h, 1), lambda: attend(h, 0))
        return carry

    lax.fori_loop(1, H, head, None)

    def attention_out(c, n):
        rows = _rows(c, n)
        sub = lax.broadcasted_iota(I32, (8, n), 0)
        parts = []
        for h in range(0, H, 2):
            even, odd = ot_buf[h, :, rows], ot_buf[h + 1, :, rows]
            even = even * (1.0 / even[VR - 1:VR])
            odd = odd * (1.0 / odd[0:1])
            parts += [even[0:16], jnp.where(sub < 4, even[16:24], odd[0:8]), odd[8:24]]
        return jnp.concatenate(parts, axis=0).T

    def project(c):
        o = attention_out(c, TM)
        x = x_buf[_rows(c, TM), :].astype(F32)
        rest = x[:, :2 * HD] + _mm(o[:, 2 * HD:].astype(BF16), wo_buf[2 * HD:, :2 * HD])
        last = x[:, 2 * HD:] + _mm(o.astype(BF16), wo_buf[:, 2 * HD:])
        h = {}
        _strassen(lambda i: _mm(_left(i, lambda r, col: o[r * HM:(r + 1) * HM, col * HD:(col + 1) * HD]).astype(BF16),
                                weights(i, so_buf, wo_block)),
                  lambda r, col: rest[r * HM:(r + 1) * HM, col * HD:(col + 1) * HD],
                  lambda r, col, val: h.update({(r, col): val}))
        return jnp.concatenate(
            [jnp.concatenate([h[r, 0], h[r, 1], last[r * HM:(r + 1) * HM]], axis=1) for r in range(2)], axis=0)

    def ffn(c, is_last):
        act = {}

        def activate(r, col, f):
            f = jnp.where(f > 0.0, f, 0.0)
            act[r, col] = f * f

        rest = _mm(xn_buf[:, 2 * HD:], w1_buf[2 * HD:, :]) + b1_buf[...].astype(F32)[None, :]
        _strassen(lambda i: _mm(normed(i), weights(i, s1_buf, w1_block)),
                  lambda r, col: rest[r * HM:(r + 1) * HM, col * HF:(col + 1) * HF], activate)
        todo, writes = [], []
        if not is_last:
            h_next = project(c + 1)
            todo = list(range(0, HM, LN_ROWS))
        b2 = b2_buf[...].astype(F32)[None, :]
        early = [_mm(act[r, 1 - r].astype(BF16), w2_buf[(1 - r) * HF:(2 - r) * HF, 2 * HD:]) for r in range(2)]
        for r in range(2):
            last = early[r] + _mm(act[r, r].astype(BF16), w2_buf[r * HF:(r + 1) * HF, 2 * HD:])
            out_buf[_rows(2 * c + r, HM), 2 * HD:] = (
                h_buf[r * HM:(r + 1) * HM, 2 * HD:] + b2[:, 2 * HD:] + last).astype(BF16)

        def product(i):
            m = _mm(_left(i, lambda r, col: act[r, col]).astype(BF16), weights(i, s2_buf, w2_block))

            def load(r):
                v = h_next[r:r + LN_ROWS]
                return jnp.concatenate([_after(c < 0, m[:LN_ROWS, :LANES], v[:, :LANES]), v[:, LANES:]], axis=1)

            for _ in range(3):
                if todo:
                    writes.extend(norm_rows(load, todo.pop(0)))
            return m

        def put_out(r, col, val):
            out_buf[_rows(2 * c + r, HM), col * HD:(col + 1) * HD] = val.astype(BF16)
            if is_last and (r, col) == (1, 0):
                for cp in last_copies[:3]:
                    cp.start()
            if is_last and r == col:
                last_copies[3 + r].start()

        _strassen(product,
                  lambda r, col: h_buf[r * HM:(r + 1) * HM, col * HD:(col + 1) * HD] + b2[:, col * HD:(col + 1) * HD],
                  put_out)
        assert not todo
        if not is_last:
            h_buf[...] = h_next
            flush(writes)

    h_first = []
    attend(H, 0, score=False, after_first_unit=lambda: h_first.append(project(0)))
    h_buf[...] = h_first[0]
    writes = []
    for r in range(0, HM, LN_ROWS):
        writes += norm_rows(lambda r0: h_first[0][r0:r0 + LN_ROWS], r)
    flush(writes)
    safe = jnp.logical_and(range_buf[0] >= SUM_MIN, range_buf[1] <= ACC_MAX)

    @pl.when(jnp.max(jnp.where(safe, 0.0, 1.0)) > 0.0)
    def _():
        lax.fori_loop(0, H * NU, attend_shifted, 0)

        def project_again(i, carry):
            rows = _rows(i, LANES)
            h_buf[rows, :] = x_buf[rows, :].astype(F32) + _mm(attention_out(i, LANES).astype(BF16), wo_buf[...])
            return carry

        def normalize_again(i, carry):
            flush(norm_rows(lambda r: h_buf[pl.ds(r, LN_ROWS), :], pl.multiple_of(i * LN_ROWS, LN_ROWS)))
            return carry

        lax.fori_loop(0, TM // LANES, project_again, 0)
        lax.fori_loop(0, HM // LN_ROWS, normalize_again, 0)

    def ffn_chunk(c, carry):
        ffn(c, False)
        out_copy(c).start()
        return carry

    lax.fori_loop(0, N_CHUNKS - 1, ffn_chunk, 0)
    ffn(N_CHUNKS - 1, True)
    for cp in [out_copy(c) for c in range(N_CHUNKS - 1)] + last_copies:
        cp.wait()


@jax.jit
def pallas_sequential_preLN__softmax_full_mha__dense_activation_squared_relu__prompt_kernel(
    A_x: jax.Array,
    A_wqkv: jax.Array,
    A_wo: jax.Array,
    B_x: jax.Array,
    B_w1: jax.Array,
    B_b1: jax.Array,
    B_w2: jax.Array,
    B_b2: jax.Array,
):
    del B_x
    any_spec = pl.BlockSpec(memory_space=pl.ANY)
    return pl.pallas_call(
        _kernel,
        out_shape=jax.ShapeDtypeStruct(A_x.shape, A_x.dtype),
        in_specs=[any_spec] * 7,
        out_specs=any_spec,
        scratch_shapes=list(_scratch_shapes().values()),
        compiler_params=pltpu.CompilerParams(
            vmem_limit_bytes=100 * 2**20,
            flags={"XLA_TPU_EVENLY_DISTRIBUTE_CRITICAL_NODES": True}),
    )(A_x, A_wqkv, A_wo, B_w1, B_b1, B_w2, B_b2)
```
